```python
import jax
import jax.numpy as jnp

def _softmax(x, axis=-1):
    return jax.nn.softmax(x, axis=axis)

def _gelu(x):
    return jax.nn.gelu(x, approximate=True)

def _silu(x):
    return jax.nn.silu(x)

def _sigmoid(x):
    return jax.nn.sigmoid(x)

def _layernorm(x, axis=-1, eps=1e-05):
    m = jnp.mean(x, axis=axis, keepdims=True)
    v = jnp.var(x, axis=axis, keepdims=True)
    return (x - m) / jnp.sqrt(v + eps)

def _scatter_add(tgt, idx, src, axis=0):
    return tgt.at[idx].add(src)

def _segment_sum(src, seg, n):
    return jax.ops.segment_sum(src, seg, n)

class _Rng:

    def __init__(self, key):
        self._k = key

    def _next(self):
        self._k, sub = jax.random.split(self._k)
        return sub

    def normal(self, shape):
        return jax.random.normal(self._next(), shape, dtype=jnp.bfloat16)

    def randint(self, lo, hi, shape):
        return jax.random.randint(self._next(), shape, lo, hi, dtype=jnp.int32)

    def uniform(self, shape, lo=0.0, hi=1.0):
        return jax.random.uniform(self._next(), shape, jnp.bfloat16, lo, hi)

    def permutation(self, n):
        return jax.random.permutation(self._next(), n)
kernel_name = 'adaLN_cond__memory_aug_recurrent_mem_tr__dense_activation_gelu__prompt'

def setup_inputs():
    _rng = _Rng(jax.random.key(int.from_bytes(__import__("os").urandom(4), "little")))
    _w = lambda a: (lambda t: t.astype(jnp.bfloat16) if jnp.issubdtype(t.dtype, jnp.floating) else t)(jnp.asarray(a))

    def _A_setup():
        B, S, Dm = (1, 2048, 1024)
        H, Dh = (32, 128)
        M, seg = (8, 32)
        seg = min(seg, S)
        S = S // seg * seg
        return {'x': _w((lambda *s: _rng.normal(s) * 0.05)(B, S, Dm)), 'mem0': _w((lambda *s: _rng.normal(s) * 0.05)(B, M, Dm)), 'Wq': _w((lambda *s: _rng.normal(s) * 0.05)(Dm, H, Dh) * Dm ** (-0.5)), 'Wk': _w((lambda *s: _rng.normal(s) * 0.05)(Dm, H, Dh) * Dm ** (-0.5)), 'Wv': _w((lambda *s: _rng.normal(s) * 0.05)(Dm, H, Dh) * Dm ** (-0.5)), 'Wo': _w((lambda *s: _rng.normal(s) * 0.05)(H, Dh, Dm) * (H * Dh) ** (-0.5)), 'seg_len': seg}
    _A_in = _A_setup()

    def _B_setup():
        B, S, D, F = (1, 2048, 1024, 3584)
        return {'x': _w((lambda *s: _rng.normal(s) * 0.05)(B, S, D)), 'w1': _w((lambda *s: _rng.normal(s) * 0.05)(D, F) * D ** (-0.5)), 'b1': _w((lambda *s: _rng.normal(s) * 0.05)(F) * 0.01), 'w2': _w((lambda *s: _rng.normal(s) * 0.05)(F, D) * F ** (-0.5)), 'b2': _w((lambda *s: _rng.normal(s) * 0.05)(D) * 0.01)}
    _B_in = _B_setup()
    return {'A_x': _A_in['x'], 'A_mem0': _A_in['mem0'], 'A_Wq': _A_in['Wq'], 'A_Wk': _A_in['Wk'], 'A_Wv': _A_in['Wv'], 'A_Wo': _A_in['Wo'], 'A_seg_len': _A_in['seg_len'], 'B_x': _B_in['x'], 'B_w1': _B_in['w1'], 'B_b1': _B_in['b1'], 'B_w2': _B_in['w2'], 'B_b2': _B_in['b2'], 'c': _w((lambda *s: _rng.normal(s) * 0.05)(1, 1024)), 'w_mod': _w((lambda *s: _rng.normal(s) * 0.05)(1024, 6 * 1024) * 1024 ** (-0.5))}

def reference(A_x, A_mem0, A_Wq, A_Wk, A_Wv, A_Wo, A_seg_len, B_x, B_w1, B_b1, B_w2, B_b2, c, w_mod):

    def _A_ref(x, mem0, Wq, Wk, Wv, Wo, seg_len):
        B, S, Dm = x.shape
        H, Dh = (Wq.shape[1], Wq.shape[2])
        M = mem0.shape[1]
        scale = Dh ** (-0.5)
        n_seg = S // seg_len
        L = M + seg_len
        idx = jnp.arange(L)
        mask = (idx[:, None] < M) | (idx[:, None] >= idx[None, :])
        mem = mem0
        outs = []
        for s in range(n_seg):
            xs = x[:, s * seg_len:(s + 1) * seg_len, :].copy()
            h = jnp.concatenate([mem, xs], axis=1)
            q = jnp.einsum('btd,dhe->bhte', h, Wq)
            k = jnp.einsum('btd,dhe->bhte', h, Wk)
            v = jnp.einsum('btd,dhe->bhte', h, Wv)
            scores = jnp.einsum('bhqe,bhke->bhqk', q, k) * scale
            scores = jnp.where(mask[None, None], scores, -1000000000.0)
            p = _softmax(scores, axis=-1)
            o = jnp.einsum('bhqk,bhke->bhqe', p, v)
            o = jnp.einsum('bhte,hed->btd', o, Wo)
            mem = o[:, :M, :].copy()
            outs.append(o[:, M:, :])
        return jnp.concatenate(outs, axis=1)

    def _B_ref(x, w1, b1, w2, b2):
        h = jnp.einsum('bsd,df->bsf', x, w1) + b1
        h = _gelu(h)
        return jnp.einsum('bsf,fd->bsd', h, w2) + b2
    x = A_x
    mod = (_silu(c) @ w_mod).reshape(c.shape[0], 6, 1, -1)
    sa, ca, ga, sb, cb, gb = (mod[:, 0].copy(), mod[:, 1].copy(), mod[:, 2].copy(), mod[:, 3].copy(), mod[:, 4].copy(), mod[:, 5].copy())
    h = _layernorm(x, axis=-1) * (1 + ca) + sa
    x = x + ga * _A_ref(h, A_mem0, A_Wq, A_Wk, A_Wv, A_Wo, A_seg_len)
    h = _layernorm(x, axis=-1) * (1 + cb) + sb
    x = x + gb * _B_ref(h, B_w1, B_b1, B_w2, B_b2)
    return x
```

```python
import functools
import math

import jax
import jax.numpy as jnp
from jax import lax
import jax.experimental.pallas as pl
import jax.experimental.pallas.tpu as pltpu

_EPS = 1e-5
_GELU_C = math.sqrt(2.0 / math.pi)


def _as_bf16(w_i32):
    return pltpu.bitcast(w_i32, jnp.bfloat16)


def _layernorm_mod(x, scale1, shift):
    m = jnp.mean(x, axis=-1, keepdims=True)
    d = x - m
    v = jnp.mean(d * d, axis=-1, keepdims=True)
    return d * lax.rsqrt(v + _EPS) * scale1 + shift


def _gelu(a):
    return 0.5 * a * (1.0 + jnp.tanh(_GELU_C * (a + 0.044715 * (a * a * a))))


def _attend(q, k, v, mask, scale):
    s = lax.dot_general(q, k, (((1,), (1,)), ((), ())),
                        preferred_element_type=jnp.float32) * scale
    s = jnp.where(mask, s, -1e9)
    m = jnp.max(s, axis=-1, keepdims=True)
    e = jnp.exp(s - m)
    p = e / jnp.sum(e, axis=-1, keepdims=True)
    return jnp.dot(p.astype(jnp.bfloat16), v, preferred_element_type=jnp.float32)


def _kernel(x_hbm, mem0_ref, wq_hbm, wk_hbm, wv_hbm, wo_hbm, w1_hbm, b1_ref,
            w2_hbm, b2_ref, c_ref, wmod_hbm, out_hbm,
            wqkv, wo, w1, w2, wmod, stage, xv, x1, keep, o_a, o_b, obuf,
            sems, ssems, osems, *, S, D, H, E, M, SEG, F, DC, NSLOT, BM, FC):
    i32, bf16, f32 = jnp.int32, jnp.bfloat16, jnp.float32
    scale = E ** -0.5
    HP = H // 2
    L = M + SEG
    G = 4

    wmod_i = wmod_hbm.bitcast(i32)
    mod_cp = [pltpu.make_async_copy(wmod_i.at[:, pl.ds(j * D, D)], wmod.at[j], sems.at[j])
              for j in range(6)]
    x_cp = pltpu.make_async_copy(x_hbm, xv, sems.at[6])
    wo_cp = pltpu.make_async_copy(wo_hbm.bitcast(i32), wo, sems.at[7])
    w1_cp = pltpu.make_async_copy(w1_hbm.bitcast(i32), w1, sems.at[8])
    w2_cp = pltpu.make_async_copy(w2_hbm.bitcast(i32), w2, sems.at[9])

    srcs = [wq_hbm.bitcast(i32), wk_hbm.bitcast(i32), wv_hbm.bitcast(i32)]
    chunks = [(t, cidx) for t in range(3) for cidx in range(D // DC)]

    def stage_cp(n):
        t, cidx = chunks[n]
        return pltpu.make_async_copy(srcs[t].at[pl.ds(cidx * DC * HP, DC * HP)],
                                     stage.at[n % NSLOT], ssems.at[n % NSLOT])

    mod_cp[0].start()
    mod_cp[1].start()
    x_cp.start()
    for n in range(NSLOT):
        stage_cp(n).start()

    cv = c_ref[...].astype(f32)
    sc = (cv * jax.nn.sigmoid(cv)).astype(bf16)

    def mod_vec(j):
        mod_cp[j].wait()
        r = jnp.dot(sc, _as_bf16(wmod[j]), preferred_element_type=f32)
        return r[0:1, :].astype(bf16).astype(f32)

    sa = mod_vec(0)
    ca1 = 1.0 + mod_vec(1)

    for n in range(len(chunks)):
        t, cidx = chunks[n]
        slot = n % NSLOT
        stage_cp(n).wait()

        def repack(hp, carry, t=t, cidx=cidx, slot=slot):
            ev = stage.at[slot][pl.ds(hp, DC // 2, stride=2 * HP), :]
            od = stage.at[slot][pl.ds(hp + HP, DC // 2, stride=2 * HP), :]
            lo = (ev & 0xFFFF) | (od << 16)
            hi = lax.shift_right_logical(ev, 16) | (od & jnp.int32(-65536))
            g = hp // (G // 2)
            i2 = hp % (G // 2)
            rows = pl.ds(cidx * DC // 2, DC // 2)
            col = pl.multiple_of((t * G + 2 * i2) * E, 2 * E)
            wqkv[g, rows, pl.ds(col, E)] = lo
            wqkv[g, rows, pl.ds(col + E, E)] = hi
            return carry

        lax.fori_loop(0, HP, repack, 0)
        if n + NSLOT < len(chunks):
            stage_cp(n + NSLOT).start()
        if n + NSLOT == len(chunks) - 1:
            wo_cp.start()
            mod_cp[2].start()
            w1_cp.start()
            w2_cp.start()
            for j in range(3, 6):
                mod_cp[j].start()

    wo_cp.wait()
    x_cp.wait()
    ga = mod_vec(2)

    ri = lax.broadcasted_iota(i32, (L, L), 0)
    ci = lax.broadcasted_iota(i32, (L, L), 1)
    mask = (ri < M) | (ri >= ci)

    def dstep(j, mem):
        base = pl.multiple_of(j * 2 * SEG, 2 * SEG)
        xb = xv[pl.ds(base, 2 * SEG), :].astype(f32)
        hb = _layernorm_mod(xb, ca1, sa)
        lhs_a = jnp.concatenate([mem, hb[0:SEG + 8]], axis=0).astype(bf16)
        for g in range(H // G):
            qkv = jnp.dot(lhs_a, _as_bf16(wqkv[g]), preferred_element_type=f32)
            keep[g] = qkv[L:L + 8]
            qkv = qkv[0:L].astype(bf16)
            for i in range(G):
                h = g * G + i
                o = _attend(qkv[:, i * E:(i + 1) * E], qkv[:, (G + i) * E:(G + i + 1) * E],
                            qkv[:, (2 * G + i) * E:(2 * G + i + 1) * E], mask, scale)
                o = o.astype(bf16)
                o_a[:, h * E:(h + 1) * E] = o[0:SEG]
                o_b[8:16, h * E:(h + 1) * E] = o[SEG:L]
        r = jnp.dot(o_a[...], _as_bf16(wo[...]), preferred_element_type=f32)
        mem_b = r[0:M]
        x1[pl.ds(base, SEG - 8), :] = (xb[0:SEG - 8] + ga * r[M:SEG]).astype(bf16)
        lhs_b = jnp.concatenate([mem_b, hb[SEG + 8:2 * SEG]], axis=0).astype(bf16)
        for g in range(H // G):
            qkv = jnp.dot(lhs_b, _as_bf16(wqkv[g]), preferred_element_type=f32)
            qkv = jnp.concatenate([qkv[0:M], keep[g], qkv[M:SEG]], axis=0).astype(bf16)
            for i in range(G):
                h = g * G + i
                o = _attend(qkv[:, i * E:(i + 1) * E], qkv[:, (G + i) * E:(G + i + 1) * E],
                            qkv[:, (2 * G + i) * E:(2 * G + i + 1) * E], mask, scale)
                o = o.astype(bf16)
                o_b[0:8, h * E:(h + 1) * E] = o[0:M]
                o_b[16:48, h * E:(h + 1) * E] = o[M:L]
        r = jnp.dot(o_b[...], _as_bf16(wo[...]), preferred_element_type=f32)
        x1[pl.ds(base + SEG - 8, SEG + 8), :] = (
            xb[SEG - 8:2 * SEG] + ga * r[M:M + SEG + 8]).astype(bf16)
        return r[0:M]

    lax.fori_loop(0, S // (2 * SEG), dstep, mem0_ref[...].astype(f32))

    sb = mod_vec(3)
    cb1 = 1.0 + mod_vec(4)
    gb = mod_vec(5)
    w1_cp.wait()
    w2_cp.wait()
    b2 = b2_ref[...].astype(f32)

    def out_cp(i, slot):
        return pltpu.make_async_copy(obuf.at[slot], out_hbm.at[pl.ds(i * BM, BM)], osems.at[slot])

    nblk = S // BM

    def mlp(i, carry):
        slot = i % 2
        base = pl.multiple_of(i * BM, BM)
        xb = x1[pl.ds(base, BM), :].astype(f32)
        h2 = _layernorm_mod(xb, cb1, sb).astype(bf16)
        acc = None
        for f in range(F // FC):
            a = jnp.dot(h2, _as_bf16(w1[:, f * FC:(f + 1) * FC]), preferred_element_type=f32)
            a = a + b1_ref[:, f * FC:(f + 1) * FC].astype(f32)
            g = _gelu(a).astype(bf16)
            y = jnp.dot(g, _as_bf16(w2[f * FC // 2:(f + 1) * FC // 2, :]),
                        preferred_element_type=f32)
            acc = y if acc is None else acc + y

        @pl.when(i >= 2)
        def _():
            out_cp(i - 2, slot).wait()

        obuf[slot] = (xb + gb * (acc + b2)).astype(bf16)
        out_cp(i, slot).start()
        return carry

    lax.fori_loop(0, nblk, mlp, 0)
    out_cp(nblk - 2, (nblk - 2) % 2).wait()
    out_cp(nblk - 1, (nblk - 1) % 2).wait()


@functools.partial(jax.jit, static_argnames=("A_seg_len",))
def pallas_adaLN_cond__memory_aug_recurrent_mem_tr__dense_activation_gelu__prompt_kernel(
    A_x, A_mem0, A_Wq, A_Wk, A_Wv, A_Wo, A_seg_len, B_x, B_w1, B_b1, B_w2, B_b2, c, w_mod,
):
    del B_x
    B, S, D = A_x.shape
    _, H, E = A_Wq.shape
    M = A_mem0.shape[1]
    F = B_w1.shape[1]
    SEG = A_seg_len
    assert B == 1 and M == 8 and SEG == 32 and S % (2 * SEG) == 0 and H % 2 == 0
    DC, NSLOT, BM, FC = 256, 4, 256, 512
    bf16, i32, f32 = jnp.bfloat16, jnp.int32, jnp.float32

    hbm = pl.BlockSpec(memory_space=pl.ANY)
    vmem = pl.BlockSpec(memory_space=pltpu.VMEM)
    kern = functools.partial(_kernel, S=S, D=D, H=H, E=E, M=M, SEG=SEG, F=F,
                             DC=DC, NSLOT=NSLOT, BM=BM, FC=FC)
    c8 = jnp.broadcast_to(c, (16, D))
    out = pl.pallas_call(
        kern,
        out_shape=jax.ShapeDtypeStruct((S, D), bf16),
        in_specs=[hbm, vmem, hbm, hbm, hbm, hbm, hbm, vmem, hbm, vmem, vmem, hbm],
        out_specs=hbm,
        scratch_shapes=[
            pltpu.VMEM((H // 4, D // 2, 12 * E), i32),
            pltpu.VMEM((H * E // 2, D), i32),
            pltpu.VMEM((D // 2, F), i32),
            pltpu.VMEM((F // 2, D), i32),
            pltpu.VMEM((6, D // 2, D), i32),
            pltpu.VMEM((NSLOT, DC * H // 2, E), i32),
            pltpu.VMEM((S, D), bf16),
            pltpu.VMEM((S, D), bf16),
            pltpu.VMEM((H // 4, 8, 12 * E), f32),
            pltpu.VMEM((SEG, H * E), bf16),
            pltpu.VMEM((SEG + 16, H * E), bf16),
            pltpu.VMEM((2, BM, D), bf16),
            pltpu.SemaphoreType.DMA((10,)),
            pltpu.SemaphoreType.DMA((NSLOT,)),
            pltpu.SemaphoreType.DMA((2,)),
        ],
        compiler_params=pltpu.CompilerParams(vmem_limit_bytes=110 * 1024 * 1024),
    )(A_x.reshape(S, D), A_mem0.reshape(M, D),
      A_Wq.reshape(D * H, E), A_Wk.reshape(D * H, E), A_Wv.reshape(D * H, E),
      A_Wo.reshape(H * E, D), B_w1, B_b1.reshape(1, F), B_w2, B_b2.reshape(1, D),
      c8, w_mod)
    return out.reshape(B, S, D)
```

```python
import functools
import math

import jax
import jax.numpy as jnp
from jax import lax
import jax.experimental.pallas as pl
import jax.experimental.pallas.tpu as pltpu

_EPS = 1e-5
_GELU_C = math.sqrt(2.0 / math.pi)


def _as_bf16(w_i32):
    return pltpu.bitcast(w_i32, jnp.bfloat16)


def _layernorm_mod(x, scale1, shift):
    m = jnp.mean(x, axis=-1, keepdims=True)
    d = x - m
    v = jnp.mean(d * d, axis=-1, keepdims=True)
    return d * lax.rsqrt(v + _EPS) * scale1 + shift


def _gelu(a):
    return 0.5 * a * (1.0 + jnp.tanh(_GELU_C * (a + 0.044715 * (a * a * a))))


def _attend(q, k, v, mask, scale):
    s = lax.dot_general(q, k, (((1,), (1,)), ((), ())),
                        preferred_element_type=jnp.float32) * scale
    s = jnp.where(mask, s, -1e9)
    m = jnp.max(s, axis=-1, keepdims=True)
    e = jnp.exp(s - m)
    p = e / jnp.sum(e, axis=-1, keepdims=True)
    return jnp.dot(p.astype(jnp.bfloat16), v, preferred_element_type=jnp.float32)


def _kernel(x_hbm, mem0_ref, wq_hbm, wk_hbm, wv_hbm, wo_hbm, w1_hbm, b1_ref,
            w2_hbm, b2_ref, c_ref, wmod_hbm, out_hbm,
            wqkv, wo, w1, w2, wmod, stage, xv, x1, hbuf, keep, o_a, o_b, obuf,
            sems, ssems, osems, *, S, D, H, E, M, SEG, F, DC, NSLOT, BM, FC):
    i32, bf16, f32 = jnp.int32, jnp.bfloat16, jnp.float32
    scale = E ** -0.5
    HP = H // 2
    L = M + SEG
    G = 4

    wmod_i = wmod_hbm.bitcast(i32)
    mod_cp = [pltpu.make_async_copy(wmod_i.at[:, pl.ds(j * D, D)], wmod.at[j], sems.at[j])
              for j in range(6)]
    x_cp = pltpu.make_async_copy(x_hbm, xv, sems.at[6])
    wo_cp = pltpu.make_async_copy(wo_hbm.bitcast(i32), wo, sems.at[7])
    w1_cp = pltpu.make_async_copy(w1_hbm.bitcast(i32), w1, sems.at[8])
    w2_cp = pltpu.make_async_copy(w2_hbm.bitcast(i32), w2, sems.at[9])

    srcs = [wq_hbm.bitcast(i32), wk_hbm.bitcast(i32), wv_hbm.bitcast(i32)]
    chunks = [(t, cidx) for t in range(3) for cidx in range(D // DC)]

    def stage_cp(n):
        t, cidx = chunks[n]
        return pltpu.make_async_copy(srcs[t].at[pl.ds(cidx * DC * HP, DC * HP)],
                                     stage.at[n % NSLOT], ssems.at[n % NSLOT])

    mod_cp[0].start()
    mod_cp[1].start()
    x_cp.start()
    for n in range(NSLOT):
        stage_cp(n).start()

    cv = c_ref[...].astype(f32)
    sc = (cv * jax.nn.sigmoid(cv)).astype(bf16)

    def mod_vec(j):
        mod_cp[j].wait()
        r = jnp.dot(sc, _as_bf16(wmod[j]), preferred_element_type=f32)
        return r[0:1, :].astype(bf16).astype(f32)

    sa = mod_vec(0)
    ca1 = 1.0 + mod_vec(1)

    for n in range(len(chunks)):
        t, cidx = chunks[n]
        slot = n % NSLOT
        stage_cp(n).wait()

        def repack(hp, carry, t=t, cidx=cidx, slot=slot):
            ev = stage.at[slot][pl.ds(hp, DC // 2, stride=2 * HP), :]
            od = stage.at[slot][pl.ds(hp + HP, DC // 2, stride=2 * HP), :]
            lo = (ev & 0xFFFF) | (od << 16)
            hi = lax.shift_right_logical(ev, 16) | (od & jnp.int32(-65536))
            g = hp // (G // 2)
            i2 = hp % (G // 2)
            rows = pl.ds(cidx * DC // 2, DC // 2)
            col = pl.multiple_of((t * G + 2 * i2) * E, 2 * E)
            wqkv[g, rows, pl.ds(col, E)] = lo
            wqkv[g, rows, pl.ds(col + E, E)] = hi
            return carry

        lax.fori_loop(0, HP, repack, 0)
        if n + NSLOT < len(chunks):
            stage_cp(n + NSLOT).start()
        if n + NSLOT == len(chunks) - 1:
            wo_cp.start()
            mod_cp[2].start()
            w1_cp.start()
            w2_cp.start()
            for j in range(3, 6):
                mod_cp[j].start()

    wo_cp.wait()
    x_cp.wait()
    ga = mod_vec(2)

    ri = lax.broadcasted_iota(i32, (L, L), 0)
    ci = lax.broadcasted_iota(i32, (L, L), 1)
    mask = (ri < M) | (ri >= ci)
    R = 2 * SEG
    nblk = S // R
    FH = F // 2

    def out_cp(i):
        return pltpu.make_async_copy(obuf.at[i % 2], out_hbm.at[pl.ds(i * R, R)], osems.at[i % 2])

    def prep_h(i):
        xb = xv[pl.ds(pl.multiple_of(i * R, R), R), :].astype(f32)
        hbuf[i % 2] = _layernorm_mod(xb, ca1, sa)

    def mlp_up(h2, f):
        a = jnp.dot(h2, _as_bf16(w1[:, f * FH:(f + 1) * FH]), preferred_element_type=f32)
        a = a + b1_ref[:, f * FH:(f + 1) * FH].astype(f32)
        return _gelu(a).astype(bf16)

    def mlp_down(g, f):
        return jnp.dot(g, _as_bf16(w2[f * FH // 2:(f + 1) * FH // 2, :]),
                       preferred_element_type=f32)

    def attn(qkv, g, store):
        for i in range(G):
            o = _attend(qkv[:, i * E:(i + 1) * E], qkv[:, (G + i) * E:(G + i + 1) * E],
                        qkv[:, (2 * G + i) * E:(2 * G + i + 1) * E], mask, scale)
            store(g * G + i, o.astype(bf16))

    def store_a(h, o):
        o_a[:, h * E:(h + 1) * E] = o[0:SEG]
        o_b[8:16, h * E:(h + 1) * E] = o[SEG:L]

    def store_b(h, o):
        o_b[0:8, h * E:(h + 1) * E] = o[0:M]
        o_b[16:48, h * E:(h + 1) * E] = o[M:L]

    def attn_pass(proj, store, fillers, early=None):
        NG = H // G
        res = []
        cur = proj(0)
        for g in range(NG):
            if g + 1 < NG:
                nxt = proj(g + 1)
            else:
                nxt = None
                res.extend(f() for f in fillers[:1])
            if g == 1 and early is not None:
                early()
            attn(cur, g, store)
            cur = nxt
        for f in fillers[1:]:
            res.append(f())
        return res

    def dstep(j, mem, with_mlp=True):
        slot = j % 2
        base = j * R if isinstance(j, int) else pl.multiple_of(j * R, R)

        if with_mlp:
            @pl.when(j >= 3)
            def _():
                out_cp(j - 3).wait()

        hb = hbuf[slot]
        st = {}

        def early():
            if with_mlp:
                xp = x1[1 - slot].astype(f32)
                st["xp"] = xp
                st["h2"] = _layernorm_mod(xp, cb1, sb).astype(bf16)
            prep_h(jnp.minimum(j + 1, nblk - 1))

        lhs_a = jnp.concatenate([mem, hb[0:SEG + 8]], axis=0).astype(bf16)
        lhs_b_rest = hb[SEG + 8:R]

        def proj_a(g):
            qkv = jnp.dot(lhs_a, _as_bf16(wqkv[g]), preferred_element_type=f32)
            keep[g] = qkv[L:L + 8]
            return qkv[0:L].astype(bf16)

        fill = [lambda: mlp_up(st["h2"], 0), lambda: mlp_up(st["h2"], 1)] if with_mlp else []
        gs = attn_pass(proj_a, store_a, fill, early)
        r = jnp.dot(o_a[...], _as_bf16(wo[...]), preferred_element_type=f32)
        if with_mlp:
            y1 = mlp_down(gs[0], 0)
        mem_b = r[0:M]
        xb = xv[pl.ds(base, R), :].astype(f32)
        x1[slot, 0:SEG - 8, :] = (xb[0:SEG - 8] + ga * r[M:SEG]).astype(bf16)
        lhs_b = jnp.concatenate([mem_b, lhs_b_rest], axis=0).astype(bf16)

        def proj_b(g):
            qkv = jnp.dot(lhs_b, _as_bf16(wqkv[g]), preferred_element_type=f32)
            return jnp.concatenate([qkv[0:M], keep[g], qkv[M:SEG]], axis=0).astype(bf16)

        fill = [lambda: mlp_down(gs[1], 1)] if with_mlp else []
        ys = attn_pass(proj_b, store_b, fill)
        if with_mlp:
            obuf[1 - slot] = (st["xp"] + gb * (y1 + ys[0] + b2)).astype(bf16)
        r = jnp.dot(o_b[...], _as_bf16(wo[...]), preferred_element_type=f32)
        x1[slot, SEG - 8:R, :] = (xb[SEG - 8:R] + ga * r[M:M + SEG + 8]).astype(bf16)
        if with_mlp:
            out_cp(j - 1).start()
        return r[0:M]

    prep_h(0)
    mem1 = dstep(0, mem0_ref[...].astype(f32), with_mlp=False)
    sb = mod_vec(3)
    cb1 = 1.0 + mod_vec(4)
    gb = mod_vec(5)
    w1_cp.wait()
    w2_cp.wait()
    b2 = b2_ref[...].astype(f32)
    lax.fori_loop(1, nblk, dstep, mem1)

    out_cp(nblk - 3).wait()
    xp = x1[(nblk - 1) % 2].astype(f32)
    h2 = _layernorm_mod(xp, cb1, sb).astype(bf16)
    y = mlp_down(mlp_up(h2, 0), 0) + mlp_down(mlp_up(h2, 1), 1)
    obuf[(nblk - 1) % 2] = (xp + gb * (y + b2)).astype(bf16)
    out_cp(nblk - 1).start()
    out_cp(nblk - 2).wait()
    out_cp(nblk - 1).wait()


@functools.partial(jax.jit, static_argnames=("A_seg_len",))
def pallas_adaLN_cond__memory_aug_recurrent_mem_tr__dense_activation_gelu__prompt_kernel(
    A_x, A_mem0, A_Wq, A_Wk, A_Wv, A_Wo, A_seg_len, B_x, B_w1, B_b1, B_w2, B_b2, c, w_mod,
):
    del B_x
    B, S, D = A_x.shape
    _, H, E = A_Wq.shape
    M = A_mem0.shape[1]
    F = B_w1.shape[1]
    SEG = A_seg_len
    assert B == 1 and M == 8 and SEG == 32 and S % (2 * SEG) == 0 and H % 2 == 0
    DC, NSLOT, BM, FC = 256, 4, 256, 512
    bf16, i32, f32 = jnp.bfloat16, jnp.int32, jnp.float32

    hbm = pl.BlockSpec(memory_space=pl.ANY)
    vmem = pl.BlockSpec(memory_space=pltpu.VMEM)
    kern = functools.partial(_kernel, S=S, D=D, H=H, E=E, M=M, SEG=SEG, F=F,
                             DC=DC, NSLOT=NSLOT, BM=BM, FC=FC)
    c8 = jnp.broadcast_to(c, (16, D))
    out = pl.pallas_call(
        kern,
        out_shape=jax.ShapeDtypeStruct((S, D), bf16),
        in_specs=[hbm, vmem, hbm, hbm, hbm, hbm, hbm, vmem, hbm, vmem, vmem, hbm],
        out_specs=hbm,
        scratch_shapes=[
            pltpu.VMEM((H // 4, D // 2, 12 * E), i32),
            pltpu.VMEM((H * E // 2, D), i32),
            pltpu.VMEM((D // 2, F), i32),
            pltpu.VMEM((F // 2, D), i32),
            pltpu.VMEM((6, D // 2, D), i32),
            pltpu.VMEM((NSLOT, DC * H // 2, E), i32),
            pltpu.VMEM((S, D), bf16),
            pltpu.VMEM((2, 2 * SEG, D), bf16),
            pltpu.VMEM((2, 2 * SEG, D), f32),
            pltpu.VMEM((H // 4, 8, 12 * E), f32),
            pltpu.VMEM((SEG, H * E), bf16),
            pltpu.VMEM((SEG + 16, H * E), bf16),
            pltpu.VMEM((2, 2 * SEG, D), bf16),
            pltpu.SemaphoreType.DMA((10,)),
            pltpu.SemaphoreType.DMA((NSLOT,)),
            pltpu.SemaphoreType.DMA((2,)),
        ],
        compiler_params=pltpu.CompilerParams(vmem_limit_bytes=110 * 1024 * 1024),
    )(A_x.reshape(S, D), A_mem0.reshape(M, D),
      A_Wq.reshape(D * H, E), A_Wk.reshape(D * H, E), A_Wv.reshape(D * H, E),
      A_Wo.reshape(H * E, D), B_w1, B_b1.reshape(1, F), B_w2, B_b2.reshape(1, D),
      c8, w_mod)
    return out.reshape(B, S, D)
```

```python
import functools
import math

import jax
import jax.numpy as jnp
from jax import lax
import jax.experimental.pallas as pl
import jax.experimental.pallas.tpu as pltpu

_EPS = 1e-5
_GELU_C = math.sqrt(2.0 / math.pi)


def _as_bf16(w_i32):
    return pltpu.bitcast(w_i32, jnp.bfloat16)


def _layernorm_mod(x, scale1, shift):
    m = jnp.mean(x, axis=-1, keepdims=True)
    d = x - m
    v = jnp.mean(d * d, axis=-1, keepdims=True)
    return d * lax.rsqrt(v + _EPS) * scale1 + shift


def _gelu(a):
    return 0.5 * a * (1.0 + jnp.tanh(_GELU_C * (a + 0.044715 * (a * a * a))))


def _attend(q, k, v, mask, scale):
    s = lax.dot_general(q, k, (((1,), (1,)), ((), ())),
                        preferred_element_type=jnp.float32) * scale
    s = jnp.where(mask, s, -1e9)
    m = jnp.max(s, axis=-1, keepdims=True)
    e = jnp.exp(s - m)
    p = e / jnp.sum(e, axis=-1, keepdims=True)
    return jnp.dot(p.astype(jnp.bfloat16), v, preferred_element_type=jnp.float32)


def _kernel(x_hbm, mem0_ref, wq_hbm, wk_hbm, wv_hbm, wo_hbm, w1_hbm, b1_ref,
            w2_hbm, b2_ref, c_ref, wmod_hbm, out_hbm,
            wqkv, wo, w1, w2, wmod, stage, xv, x1, hbuf, keep, o_a, o_b, obuf, otail,
            sems, ssems, osems, *, S, D, H, E, M, SEG, F, DC, NSLOT, LAG):
    i32, bf16, f32 = jnp.int32, jnp.bfloat16, jnp.float32
    scale = E ** -0.5
    HP = H // 2
    L = M + SEG
    G = 4

    wmod_i = wmod_hbm.bitcast(i32)
    mod_cp = [pltpu.make_async_copy(wmod_i.at[:, pl.ds(j * D, D)], wmod.at[j], sems.at[j])
              for j in range(6)]
    X0 = 256
    x_cp = pltpu.make_async_copy(x_hbm.at[pl.ds(0, X0)], xv.at[pl.ds(0, X0)], sems.at[6])
    x2_cp = pltpu.make_async_copy(x_hbm.at[pl.ds(X0, S - X0)], xv.at[pl.ds(X0, S - X0)],
                                  sems.at[10])
    wo_cp = pltpu.make_async_copy(wo_hbm.bitcast(i32), wo, sems.at[7])
    w1_cp = pltpu.make_async_copy(w1_hbm.bitcast(i32), w1, sems.at[8])
    w2_cp = pltpu.make_async_copy(w2_hbm.bitcast(i32), w2, sems.at[9])

    srcs = [wq_hbm.bitcast(i32), wk_hbm.bitcast(i32), wv_hbm.bitcast(i32)]
    chunks = [(t, cidx) for t in range(3) for cidx in range(D // DC)]

    def stage_cp(n):
        t, cidx = chunks[n]
        return pltpu.make_async_copy(srcs[t].at[pl.ds(cidx * DC * HP, DC * HP)],
                                     stage.at[n % NSLOT], ssems.at[n % NSLOT])

    mod_cp[0].start()
    mod_cp[1].start()
    x_cp.start()
    for n in range(NSLOT):
        stage_cp(n).start()

    cv = c_ref[...].astype(f32)
    sc = (cv * jax.nn.sigmoid(cv)).astype(bf16)

    def mod_vec(j):
        mod_cp[j].wait()
        r = jnp.dot(sc, _as_bf16(wmod[j]), preferred_element_type=f32)
        return r[0:1, :].astype(bf16).astype(f32)

    sa = mod_vec(0)
    ca1 = 1.0 + mod_vec(1)

    for n in range(len(chunks)):
        t, cidx = chunks[n]
        slot = n % NSLOT
        stage_cp(n).wait()

        def repack(hp, carry, t=t, cidx=cidx, slot=slot):
            ev = stage.at[slot][pl.ds(hp, DC // 2, stride=2 * HP), :]
            od = stage.at[slot][pl.ds(hp + HP, DC // 2, stride=2 * HP), :]
            lo = (ev & 0xFFFF) | (od << 16)
            hi = lax.shift_right_logical(ev, 16) | (od & jnp.int32(-65536))
            g = hp // (G // 2)
            i2 = hp % (G // 2)
            rows = pl.ds(cidx * DC // 2, DC // 2)
            col = pl.multiple_of((t * G + 2 * i2) * E, 2 * E)
            wqkv[g, rows, pl.ds(col, E)] = lo
            wqkv[g, rows, pl.ds(col + E, E)] = hi
            return carry

        lax.fori_loop(0, HP, repack, 0)
        if n + NSLOT < len(chunks):
            stage_cp(n + NSLOT).start()
        if n + NSLOT == len(chunks) - 1:
            wo_cp.start()
            mod_cp[2].start()
            x2_cp.start()
            w1_cp.start()
            w2_cp.start()
            for j in range(3, 6):
                mod_cp[j].start()

    wo_cp.wait()
    x_cp.wait()
    ga = mod_vec(2)

    ri = lax.broadcasted_iota(i32, (L, L), 0)
    ci = lax.broadcasted_iota(i32, (L, L), 1)
    mask = (ri < M) | (ri >= ci)
    R = 2 * SEG
    nblk = S // R
    FH = F // 2

    def out_cp(i):
        return pltpu.make_async_copy(obuf.at[i % 2], out_hbm.at[pl.ds(i * R, R)], osems.at[i % 2])

    def prep_h(i):
        xb = xv[pl.ds(pl.multiple_of(i * R, R), R), :].astype(f32)
        hbuf[i % 2] = _layernorm_mod(xb, ca1, sa)

    def mlp_up(h2, f):
        a = jnp.dot(h2, _as_bf16(w1[:, f * FH:(f + 1) * FH]), preferred_element_type=f32)
        a = a + b1_ref[:, f * FH:(f + 1) * FH].astype(f32)
        return _gelu(a).astype(bf16)

    def mlp_down(g, f):
        return jnp.dot(g, _as_bf16(w2[f * FH // 2:(f + 1) * FH // 2, :]),
                       preferred_element_type=f32)

    def attn(qkv, g, store):
        for i in range(G):
            o = _attend(qkv[:, i * E:(i + 1) * E], qkv[:, (G + i) * E:(G + i + 1) * E],
                        qkv[:, (2 * G + i) * E:(2 * G + i + 1) * E], mask, scale)
            store(g * G + i, o.astype(bf16))

    def store_a(h, o):
        o_a[:, h * E:(h + 1) * E] = o[0:SEG]
        o_b[8:16, h * E:(h + 1) * E] = o[SEG:L]

    def store_b(h, o):
        o_b[0:8, h * E:(h + 1) * E] = o[0:M]
        o_b[16:48, h * E:(h + 1) * E] = o[M:L]

    def attn_pass(proj, store, fillers, early=None):
        NG = H // G
        res = []
        cur = proj(0)
        for g in range(NG):
            if g + 1 < NG:
                nxt = proj(g + 1)
            else:
                nxt = None
                res.extend(f() for f in fillers[:1])
            if g == 1 and early is not None:
                early()
            attn(cur, g, store)
            cur = nxt
        for f in fillers[1:]:
            res.append(f())
        return res

    def dstep(j, mem, with_mlp=True):
        slot = j % 2
        xs = j % (LAG + 1)
        xq = (j + 1) % (LAG + 1)
        base = j * R if isinstance(j, int) else pl.multiple_of(j * R, R)

        if with_mlp:
            @pl.when(j >= LAG + 2)
            def _():
                out_cp(j - LAG - 2).wait()

        hb = hbuf[slot]
        st = {}

        def early():
            if with_mlp:
                xp = x1[xq].astype(f32)
                st["xp"] = xp
                st["h2"] = _layernorm_mod(xp, cb1, sb).astype(bf16)
            prep_h(jnp.minimum(j + 1, nblk - 1))

        lhs_a = jnp.concatenate([mem, hb[0:SEG + 8]], axis=0).astype(bf16)
        lhs_b_rest = hb[SEG + 8:R]

        def proj_a(g):
            qkv = jnp.dot(lhs_a, _as_bf16(wqkv[g]), preferred_element_type=f32)
            keep[g] = qkv[L:L + 8]
            return qkv[0:L].astype(bf16)

        fill = [lambda: mlp_up(st["h2"], 0), lambda: mlp_up(st["h2"], 1)] if with_mlp else []
        gs = attn_pass(proj_a, store_a, fill, early)
        r = jnp.dot(o_a[...], _as_bf16(wo[...]), preferred_element_type=f32)
        if with_mlp:
            y1 = mlp_down(gs[0], 0)
        mem_b = r[0:M]
        xb = xv[pl.ds(base, R), :].astype(f32)
        x1[xs, 0:SEG - 8, :] = (xb[0:SEG - 8] + ga * r[M:SEG]).astype(bf16)
        lhs_b = jnp.concatenate([mem_b, lhs_b_rest], axis=0).astype(bf16)

        def proj_b(g):
            qkv = jnp.dot(lhs_b, _as_bf16(wqkv[g]), preferred_element_type=f32)
            return jnp.concatenate([qkv[0:M], keep[g], qkv[M:SEG]], axis=0).astype(bf16)

        fill = [lambda: mlp_down(gs[1], 1)] if with_mlp else []
        ys = attn_pass(proj_b, store_b, fill)
        if with_mlp:
            obuf[(j - LAG) % 2] = (st["xp"] + gb * (y1 + ys[0] + b2)).astype(bf16)
        r = jnp.dot(o_b[...], _as_bf16(wo[...]), preferred_element_type=f32)
        x1[xs, SEG - 8:R, :] = (xb[SEG - 8:R] + ga * r[M:M + SEG + 8]).astype(bf16)
        if with_mlp:
            out_cp(j - LAG).start()
        return r[0:M]

    prep_h(0)
    mem1 = lax.fori_loop(0, LAG, lambda j, m: dstep(j, m, with_mlp=False),
                         mem0_ref[...].astype(f32))
    sb = mod_vec(3)
    cb1 = 1.0 + mod_vec(4)
    gb = mod_vec(5)
    w1_cp.wait()
    w2_cp.wait()
    x2_cp.wait()
    b2 = b2_ref[...].astype(f32)
    lax.fori_loop(LAG, nblk, dstep, mem1)

    out_cp(nblk - LAG - 2).wait()
    out_cp(nblk - LAG - 1).wait()
    tail = list(range(nblk - LAG, nblk))
    xp = jnp.concatenate([x1[i % (LAG + 1)] for i in tail], axis=0).astype(f32)
    h2 = _layernorm_mod(xp, cb1, sb).astype(bf16)
    y = mlp_down(mlp_up(h2, 0), 0) + mlp_down(mlp_up(h2, 1), 1)
    otail[...] = (xp + gb * (y + b2)).astype(bf16)
    cp = pltpu.make_async_copy(otail, out_hbm.at[pl.ds((nblk - LAG) * R, LAG * R)], osems.at[0])
    cp.start()
    cp.wait()


@functools.partial(jax.jit, static_argnames=("A_seg_len",))
def pallas_adaLN_cond__memory_aug_recurrent_mem_tr__dense_activation_gelu__prompt_kernel(
    A_x, A_mem0, A_Wq, A_Wk, A_Wv, A_Wo, A_seg_len, B_x, B_w1, B_b1, B_w2, B_b2, c, w_mod,
):
    del B_x
    B, S, D = A_x.shape
    _, H, E = A_Wq.shape
    M = A_mem0.shape[1]
    F = B_w1.shape[1]
    SEG = A_seg_len
    assert B == 1 and M == 8 and SEG == 32 and S % (2 * SEG) == 0 and H % 2 == 0
    DC, NSLOT, LAG = 256, 4, 3
    bf16, i32, f32 = jnp.bfloat16, jnp.int32, jnp.float32

    hbm = pl.BlockSpec(memory_space=pl.ANY)
    vmem = pl.BlockSpec(memory_space=pltpu.VMEM)
    kern = functools.partial(_kernel, S=S, D=D, H=H, E=E, M=M, SEG=SEG, F=F,
                             DC=DC, NSLOT=NSLOT, LAG=LAG)
    c8 = jnp.broadcast_to(c, (16, D))
    out = pl.pallas_call(
        kern,
        out_shape=jax.ShapeDtypeStruct((S, D), bf16),
        in_specs=[hbm, vmem, hbm, hbm, hbm, hbm, hbm, vmem, hbm, vmem, vmem, hbm],
        out_specs=hbm,
        scratch_shapes=[
            pltpu.VMEM((H // 4, D // 2, 12 * E), i32),
            pltpu.VMEM((H * E // 2, D), i32),
            pltpu.VMEM((D // 2, F), i32),
            pltpu.VMEM((F // 2, D), i32),
            pltpu.VMEM((6, D // 2, D), i32),
            pltpu.VMEM((NSLOT, DC * H // 2, E), i32),
            pltpu.VMEM((S, D), bf16),
            pltpu.VMEM((LAG + 1, 2 * SEG, D), bf16),
            pltpu.VMEM((2, 2 * SEG, D), f32),
            pltpu.VMEM((H // 4, 8, 12 * E), f32),
            pltpu.VMEM((SEG, H * E), bf16),
            pltpu.VMEM((SEG + 16, H * E), bf16),
            pltpu.VMEM((2, 2 * SEG, D), bf16),
            pltpu.VMEM((LAG * 2 * SEG, D), bf16),
            pltpu.SemaphoreType.DMA((11,)),
            pltpu.SemaphoreType.DMA((NSLOT,)),
            pltpu.SemaphoreType.DMA((2,)),
        ],
        compiler_params=pltpu.CompilerParams(vmem_limit_bytes=110 * 1024 * 1024),
    )(A_x.reshape(S, D), A_mem0.reshape(M, D),
      A_Wq.reshape(D * H, E), A_Wk.reshape(D * H, E), A_Wv.reshape(D * H, E),
      A_Wo.reshape(H * E, D), B_w1, B_b1.reshape(1, F), B_w2, B_b2.reshape(1, D),
      c8, w_mod)
    return out.reshape(B, S, D)
```

```python
import functools
import math

import jax
import jax.numpy as jnp
from jax import lax
import jax.experimental.pallas as pl
import jax.experimental.pallas.tpu as pltpu

_EPS = 1e-5
_GELU_C = math.sqrt(2.0 / math.pi)


def _as_bf16(w_i32):
    return pltpu.bitcast(w_i32, jnp.bfloat16)


def _layernorm_mod(x, scale1, shift):
    m = jnp.mean(x, axis=-1, keepdims=True)
    d = x - m
    v = jnp.mean(d * d, axis=-1, keepdims=True)
    return d * lax.rsqrt(v + _EPS) * scale1 + shift


def _gelu(a):
    return 0.5 * a * (1.0 + jnp.tanh(_GELU_C * (a + 0.044715 * (a * a * a))))


def _attend(q, k, v, mask, scale):
    s = lax.dot_general(q, k, (((1,), (1,)), ((), ())),
                        preferred_element_type=jnp.float32) * scale
    s = jnp.where(mask, s, -1e9)
    m = jnp.max(s, axis=-1, keepdims=True)
    e = jnp.exp(s - m)
    p = e / jnp.sum(e, axis=-1, keepdims=True)
    return jnp.dot(p.astype(jnp.bfloat16), v, preferred_element_type=jnp.float32)


def _kernel(x_hbm, x3_hbm, mem0_ref, wq_hbm, wk_hbm, wv_hbm, wo_hbm, w1_hbm, b1_ref,
            w2_hbm, b2_ref, c_ref, wmod_hbm, out_hbm,
            wqkv, wo, w1, w2, wmod, stage, xv, x1, hbuf, xpre, hpre, pre, o_a, o_b, obuf, otail,
            sems, ssems, osems, *, S, D, H, E, M, SEG, F, DC, NSLOT, LAG):
    i32, bf16, f32 = jnp.int32, jnp.bfloat16, jnp.float32
    scale = E ** -0.5
    HP = H // 2
    L = M + SEG
    G = 4

    wmod_i = wmod_hbm.bitcast(i32)
    mod_cp = [pltpu.make_async_copy(wmod_i.at[:, pl.ds(j * D, D)], wmod.at[j], sems.at[j])
              for j in range(6)]
    x_cp = pltpu.make_async_copy(x_hbm, xv, sems.at[6])
    wo_cp = pltpu.make_async_copy(wo_hbm.bitcast(i32), wo, sems.at[7])
    w1_cp = pltpu.make_async_copy(w1_hbm.bitcast(i32), w1, sems.at[8])
    w2_cp = pltpu.make_async_copy(w2_hbm.bitcast(i32), w2, sems.at[9])

    srcs = [wq_hbm.bitcast(i32), wk_hbm.bitcast(i32), wv_hbm.bitcast(i32)]
    chunks = [(t, cidx) for t in range(3) for cidx in range(D // DC)]

    def stage_cp(n):
        t, cidx = chunks[n]
        return pltpu.make_async_copy(srcs[t].at[pl.ds(cidx * DC * HP, DC * HP)],
                                     stage.at[n % NSLOT], ssems.at[n % NSLOT])

    NS = S // SEG
    PB = NS * 8
    xb_cp = pltpu.make_async_copy(x3_hbm.at[:, pl.ds(SEG - 8, 8), :], xpre, sems.at[11])
    xb_cp.start()
    mod_cp[0].start()
    mod_cp[1].start()
    for n in range(NSLOT):
        stage_cp(n).start()

    cv = c_ref[...].astype(f32)
    sc = (cv * jax.nn.sigmoid(cv)).astype(bf16)

    def mod_vec(j):
        mod_cp[j].wait()
        r = jnp.dot(sc, _as_bf16(wmod[j]), preferred_element_type=f32)
        return r[0:1, :].astype(bf16).astype(f32)

    sa = mod_vec(0)
    ca1 = 1.0 + mod_vec(1)
    xb_cp.wait()
    hpre[...] = _layernorm_mod(xpre[...].reshape(PB, D).astype(f32), ca1, sa).astype(bf16)

    per = D // DC
    for n in range(len(chunks)):
        t, cidx = chunks[n]
        slot = n % NSLOT
        stage_cp(n).wait()

        def repack(hp, carry, t=t, cidx=cidx, slot=slot):
            ev = stage.at[slot][pl.ds(hp, DC // 2, stride=2 * HP), :]
            od = stage.at[slot][pl.ds(hp + HP, DC // 2, stride=2 * HP), :]
            lo = (ev & 0xFFFF) | (od << 16)
            hi = lax.shift_right_logical(ev, 16) | (od & jnp.int32(-65536))
            g = hp // (G // 2)
            i2 = hp % (G // 2)
            rows = pl.ds(cidx * DC // 2, DC // 2)
            col = pl.multiple_of((t * G + 2 * i2) * E, 2 * E)
            wqkv[g, rows, pl.ds(col, E)] = lo
            wqkv[g, rows, pl.ds(col + E, E)] = hi
            return carry

        lax.fori_loop(0, HP, repack, 0)
        if n + NSLOT < len(chunks):
            stage_cp(n + NSLOT).start()
        if n == per - 1:
            x_cp.start()
            wo_cp.start()
            mod_cp[2].start()
        if n == 2 * per - 1:
            w1_cp.start()
            w2_cp.start()
            for j in range(3, 6):
                mod_cp[j].start()
        if n % per == per - 1:
            W = G * E

            def bulk(g, carry, t=t):
                pre[g, :, pl.ds(t * W, W)] = jnp.dot(
                    hpre[...], _as_bf16(wqkv[g, :, t * W:(t + 1) * W]),
                    preferred_element_type=f32).astype(bf16)
                return carry

            lax.fori_loop(0, H // G, bulk, 0)

    wo_cp.wait()
    x_cp.wait()
    ga = mod_vec(2)

    ri = lax.broadcasted_iota(i32, (L, L), 0)
    ci = lax.broadcasted_iota(i32, (L, L), 1)
    mask = (ri < M) | (ri >= ci)
    R = 2 * SEG
    nblk = S // R
    FH = F // 2

    def out_cp(i):
        return pltpu.make_async_copy(obuf.at[i % 2], out_hbm.at[pl.ds(i * R, R)], osems.at[i % 2])

    def prep_h(i):
        xb = xv[pl.ds(pl.multiple_of(i * R, R), R), :].astype(f32)
        hbuf[i % 2] = _layernorm_mod(xb, ca1, sa)

    def mlp_up(h2, f):
        a = jnp.dot(h2, _as_bf16(w1[:, f * FH:(f + 1) * FH]), preferred_element_type=f32)
        a = a + b1_ref[:, f * FH:(f + 1) * FH].astype(f32)
        return _gelu(a).astype(bf16)

    def mlp_down(g, f):
        return jnp.dot(g, _as_bf16(w2[f * FH // 2:(f + 1) * FH // 2, :]),
                       preferred_element_type=f32)

    def attn(qkv, g, store):
        for i in range(G):
            o = _attend(qkv[:, i * E:(i + 1) * E], qkv[:, (G + i) * E:(G + i + 1) * E],
                        qkv[:, (2 * G + i) * E:(2 * G + i + 1) * E], mask, scale)
            store(g * G + i, o.astype(bf16))

    def store_a(h, o):
        o_a[:, h * E:(h + 1) * E] = o[0:SEG]
        o_b[8:16, h * E:(h + 1) * E] = o[SEG:L]

    def store_b(h, o):
        o_b[0:8, h * E:(h + 1) * E] = o[0:M]
        o_b[16:48, h * E:(h + 1) * E] = o[M:L]

    def attn_pass(proj, store, fillers, early=None):
        NG = H // G
        res = []
        cur = proj(0)
        for g in range(NG):
            if g + 1 < NG:
                nxt = proj(g + 1)
            else:
                nxt = None
                res.extend(f() for f in fillers[:1])
            if g == 1 and early is not None:
                early()
            attn(cur, g, store)
            cur = nxt
        for f in fillers[1:]:
            res.append(f())
        return res

    def dstep(j, mem, with_mlp=True):
        slot = j % 2
        xs = j % (LAG + 1)
        xq = (j + 1) % (LAG + 1)
        base = j * R if isinstance(j, int) else pl.multiple_of(j * R, R)

        if with_mlp:
            @pl.when(j >= LAG + 2)
            def _():
                out_cp(j - LAG - 2).wait()

        hb = hbuf[slot]
        st = {}

        def early():
            if with_mlp:
                xp = x1[xq].astype(f32)
                st["xp"] = xp
                st["h2"] = _layernorm_mod(xp, cb1, sb).astype(bf16)
            prep_h(jnp.minimum(j + 1, nblk - 1))

        lhs_a = jnp.concatenate([mem, hb[0:SEG - 8]], axis=0).astype(bf16)
        lhs_b_rest = hb[SEG:R - 8]
        p0 = j * 16 if isinstance(j, int) else pl.multiple_of(j * 16, 16)

        def proj(lhs, g, off):
            qkv = jnp.dot(lhs, _as_bf16(wqkv[g]), preferred_element_type=f32).astype(bf16)
            return jnp.concatenate([qkv, pre[g, pl.ds(p0 + off, 8), :]], axis=0)

        proj_a = lambda g: proj(lhs_a, g, 0)

        fill = [lambda: mlp_up(st["h2"], 0), lambda: mlp_up(st["h2"], 1)] if with_mlp else []
        gs = attn_pass(proj_a, store_a, fill, early)
        r = jnp.dot(o_a[...], _as_bf16(wo[...]), preferred_element_type=f32)
        if with_mlp:
            y1 = mlp_down(gs[0], 0)
        mem_b = r[0:M]
        xb = xv[pl.ds(base, R), :].astype(f32)
        x1[xs, 0:SEG - 8, :] = (xb[0:SEG - 8] + ga * r[M:SEG]).astype(bf16)
        lhs_b = jnp.concatenate([mem_b, lhs_b_rest], axis=0).astype(bf16)

        proj_b = lambda g: proj(lhs_b, g, 8)
        fill = [lambda: mlp_down(gs[1], 1)] if with_mlp else []
        ys = attn_pass(proj_b, store_b, fill)
        if with_mlp:
            obuf[(j - LAG) % 2] = (st["xp"] + gb * (y1 + ys[0] + b2)).astype(bf16)
        r = jnp.dot(o_b[...], _as_bf16(wo[...]), preferred_element_type=f32)
        x1[xs, SEG - 8:R, :] = (xb[SEG - 8:R] + ga * r[M:M + SEG + 8]).astype(bf16)
        if with_mlp:
            out_cp(j - LAG).start()
        return r[0:M]

    prep_h(0)
    mem1 = lax.fori_loop(0, LAG, lambda j, m: dstep(j, m, with_mlp=False),
                         mem0_ref[...].astype(f32))
    sb = mod_vec(3)
    cb1 = 1.0 + mod_vec(4)
    gb = mod_vec(5)
    w1_cp.wait()
    w2_cp.wait()
    b2 = b2_ref[...].astype(f32)
    lax.fori_loop(LAG, nblk, dstep, mem1)

    out_cp(nblk - LAG - 2).wait()
    out_cp(nblk - LAG - 1).wait()
    tail = list(range(nblk - LAG, nblk))
    xp = jnp.concatenate([x1[i % (LAG + 1)] for i in tail], axis=0).astype(f32)
    h2 = _layernorm_mod(xp, cb1, sb).astype(bf16)
    y = mlp_down(mlp_up(h2, 0), 0) + mlp_down(mlp_up(h2, 1), 1)
    otail[...] = (xp + gb * (y + b2)).astype(bf16)
    cp = pltpu.make_async_copy(otail, out_hbm.at[pl.ds((nblk - LAG) * R, LAG * R)], osems.at[0])
    cp.start()
    cp.wait()


@functools.partial(jax.jit, static_argnames=("A_seg_len",))
def pallas_adaLN_cond__memory_aug_recurrent_mem_tr__dense_activation_gelu__prompt_kernel(
    A_x, A_mem0, A_Wq, A_Wk, A_Wv, A_Wo, A_seg_len, B_x, B_w1, B_b1, B_w2, B_b2, c, w_mod,
):
    del B_x
    B, S, D = A_x.shape
    _, H, E = A_Wq.shape
    M = A_mem0.shape[1]
    F = B_w1.shape[1]
    SEG = A_seg_len
    assert B == 1 and M == 8 and SEG == 32 and S % (2 * SEG) == 0 and H % 2 == 0
    DC, NSLOT, LAG = 256, 4, 1
    bf16, i32, f32 = jnp.bfloat16, jnp.int32, jnp.float32

    hbm = pl.BlockSpec(memory_space=pl.ANY)
    vmem = pl.BlockSpec(memory_space=pltpu.VMEM)
    kern = functools.partial(_kernel, S=S, D=D, H=H, E=E, M=M, SEG=SEG, F=F,
                             DC=DC, NSLOT=NSLOT, LAG=LAG)
    c8 = jnp.broadcast_to(c, (16, D))
    out = pl.pallas_call(
        kern,
        out_shape=jax.ShapeDtypeStruct((S, D), bf16),
        in_specs=[hbm, hbm, vmem, hbm, hbm, hbm, hbm, hbm, vmem, hbm, vmem, vmem, hbm],
        out_specs=hbm,
        scratch_shapes=[
            pltpu.VMEM((H // 4, D // 2, 12 * E), i32),
            pltpu.VMEM((H * E // 2, D), i32),
            pltpu.VMEM((D // 2, F), i32),
            pltpu.VMEM((F // 2, D), i32),
            pltpu.VMEM((6, D // 2, D), i32),
            pltpu.VMEM((NSLOT, DC * H // 2, E), i32),
            pltpu.VMEM((S, D), bf16),
            pltpu.VMEM((LAG + 1, 2 * SEG, D), bf16),
            pltpu.VMEM((2, 2 * SEG, D), f32),
            pltpu.VMEM((S // SEG, 8, D), bf16),
            pltpu.VMEM((S // SEG * 8, D), bf16),
            pltpu.VMEM((H // 4, S // SEG * 8, 12 * E), bf16),
            pltpu.VMEM((SEG, H * E), bf16),
            pltpu.VMEM((SEG + 16, H * E), bf16),
            pltpu.VMEM((2, 2 * SEG, D), bf16),
            pltpu.VMEM((LAG * 2 * SEG, D), bf16),
            pltpu.SemaphoreType.DMA((12,)),
            pltpu.SemaphoreType.DMA((NSLOT,)),
            pltpu.SemaphoreType.DMA((2,)),
        ],
        compiler_params=pltpu.CompilerParams(vmem_limit_bytes=110 * 1024 * 1024),
    )(A_x.reshape(S, D), A_x.reshape(S // SEG, SEG, D), A_mem0.reshape(M, D),
      A_Wq.reshape(D * H, E), A_Wk.reshape(D * H, E), A_Wv.reshape(D * H, E),
      A_Wo.reshape(H * E, D), B_w1, B_b1.reshape(1, F), B_w2, B_b2.reshape(1, D),
      c8, w_mod)
    return out.reshape(B, S, D)
```

```python
import functools
import math

import jax
import jax.numpy as jnp
from jax import lax
import jax.experimental.pallas as pl
import jax.experimental.pallas.tpu as pltpu

_EPS = 1e-5
_GELU_C = math.sqrt(2.0 / math.pi)


def _as_bf16(w_i32):
    return pltpu.bitcast(w_i32, jnp.bfloat16)


def _layernorm_mod(x, scale1, shift):
    m = jnp.mean(x, axis=-1, keepdims=True)
    d = x - m
    v = jnp.mean(d * d, axis=-1, keepdims=True)
    return d * lax.rsqrt(v + _EPS) * scale1 + shift


def _gelu(a):
    return 0.5 * a * (1.0 + jnp.tanh(_GELU_C * (a + 0.044715 * (a * a * a))))


def _attend(q, k, v, mask, scale):
    s = lax.dot_general(q, k, (((1,), (1,)), ((), ())),
                        preferred_element_type=jnp.float32) * scale
    s = jnp.where(mask, s, -1e9)
    m = jnp.max(s, axis=-1, keepdims=True)
    e = jnp.exp(s - m)
    p = e / jnp.sum(e, axis=-1, keepdims=True)
    return jnp.dot(p.astype(jnp.bfloat16), v, preferred_element_type=jnp.float32)


def _kernel(x_hbm, x3_hbm, mem0_ref, wq_hbm, wk_hbm, wv_hbm, wo_hbm, w1_hbm, b1_ref,
            w2_hbm, b2_ref, c_ref, wmod_hbm, out_hbm,
            wq, wk, wv, wo, w1, w2, wmod, stage, xv, x1, hbuf, xpre, hpre, pre, o_a, o_b, obuf, otail,
            sems, ssems, osems, *, S, D, H, E, M, SEG, F, DC, NSLOT, LAG):
    i32, bf16, f32 = jnp.int32, jnp.bfloat16, jnp.float32
    scale = E ** -0.5
    HP = H // 2
    L = M + SEG
    G = 4

    wmod_i = wmod_hbm.bitcast(i32)
    mod_cp = [pltpu.make_async_copy(wmod_i.at[:, pl.ds(j * D, D)], wmod.at[j], sems.at[j])
              for j in range(6)]
    x_cp = pltpu.make_async_copy(x_hbm, xv, sems.at[6])
    wo_cp = pltpu.make_async_copy(wo_hbm.bitcast(i32), wo, sems.at[7])
    w1_cp = pltpu.make_async_copy(w1_hbm.bitcast(i32), w1, sems.at[8])
    w2_cp = pltpu.make_async_copy(w2_hbm.bitcast(i32), w2, sems.at[9])

    srcs = [wq_hbm.bitcast(i32), wk_hbm.bitcast(i32), wv_hbm.bitcast(i32)]
    chunks = [(t, cidx) for t in range(3) for cidx in range(D // DC)]

    def stage_cp(n):
        t, cidx = chunks[n]
        return pltpu.make_async_copy(srcs[t].at[pl.ds(cidx * DC * HP, DC * HP)],
                                     stage.at[n % NSLOT], ssems.at[n % NSLOT])

    NS = S // SEG
    PB = NS * 8
    xb_cp = pltpu.make_async_copy(x3_hbm.at[:, pl.ds(SEG - 8, 8), :], xpre, sems.at[11])
    xb_cp.start()
    mod_cp[0].start()
    mod_cp[1].start()
    for n in range(NSLOT):
        stage_cp(n).start()

    cv = c_ref[...].astype(f32)
    sc = (cv * jax.nn.sigmoid(cv)).astype(bf16)

    def mod_vec(j):
        mod_cp[j].wait()
        r = jnp.dot(sc, _as_bf16(wmod[j]), preferred_element_type=f32)
        return r[0:1, :].astype(bf16).astype(f32)

    sa = mod_vec(0)
    ca1 = 1.0 + mod_vec(1)
    xb_cp.wait()
    hpre[...] = pltpu.bitcast(
        _layernorm_mod(xpre[...].reshape(PB, D).astype(f32), ca1, sa).astype(bf16), i32)
    wts = ((wq.at[0], wq.at[1]), (wk.at[0], wk.at[1]), (wv.at[0], wv.at[1]))

    per = D // DC
    W = G * E

    PITCH = D // 2 + 8

    def repack(n):
        t, cidx = chunks[n]
        slot = n % NSLOT
        stage_cp(n).wait()
        w_even, w_odd = wts[t]

        def body(q, carry):
            for u in range(8):
                pp = q * 8 + u
                a = stage[slot, pl.ds(pl.multiple_of(pp * 2 * HP, 2 * HP), HP), :]
                b = stage[slot, pl.ds(pl.multiple_of(pp * 2 * HP + HP, HP), HP), :]
                lo = (a & 0xFFFF) | (b << 16)
                hi = lax.shift_right_logical(a, 16) | (b & jnp.int32(-65536))
                dst = pl.ds(cidx * DC // 2 + pp, HP, stride=PITCH)
                w_even[dst, :] = lo
                w_odd[dst, :] = hi
            return carry

        lax.fori_loop(0, DC // 16, body, 0)
        if n + NSLOT < len(chunks):
            stage_cp(n + NSLOT).start()

    def wgroup(t, g):
        w_even, w_odd = wts[t]
        parts = []
        for i in range(G // 2):
            hp = g * (G // 2) + i
            r0 = hp * PITCH if isinstance(hp, int) else pl.multiple_of(hp * PITCH, 8)
            parts += [w_even[pl.ds(r0, D // 2), :], w_odd[pl.ds(r0, D // 2), :]]
        return parts

    for t in range(3):
        for n in range(t * per, (t + 1) * per):
            repack(n)
        if t == 0:
            x_cp.start()
            wo_cp.start()
            mod_cp[2].start()
        if t == 1:
            w1_cp.start()
            w2_cp.start()
            for j in range(3, 6):
                mod_cp[j].start()

        def bulk(g, carry, t=t):
            w = jnp.concatenate(wgroup(t, g), axis=1)
            pre[g, :, pl.ds(t * W, W)] = jnp.dot(
                _as_bf16(hpre[...]), _as_bf16(w), preferred_element_type=f32).astype(bf16)
            return carry

        lax.fori_loop(0, H // G, bulk, 0)

    wo_cp.wait()
    x_cp.wait()
    ga = mod_vec(2)

    ri = lax.broadcasted_iota(i32, (L, L), 0)
    ci = lax.broadcasted_iota(i32, (L, L), 1)
    mask = (ri < M) | (ri >= ci)
    R = 2 * SEG
    nblk = S // R
    FH = F // 2

    def out_cp(i):
        return pltpu.make_async_copy(obuf.at[i % 2], out_hbm.at[pl.ds(i * R, R)], osems.at[i % 2])

    def prep_h(i):
        xb = xv[pl.ds(pl.multiple_of(i * R, R), R), :].astype(f32)
        hbuf[i % 2] = _layernorm_mod(xb, ca1, sa)

    def mlp_up(h2, f):
        a = jnp.dot(h2, _as_bf16(w1[:, f * FH:(f + 1) * FH]), preferred_element_type=f32)
        a = a + b1_ref[:, f * FH:(f + 1) * FH].astype(f32)
        return _gelu(a).astype(bf16)

    def mlp_down(g, f):
        return jnp.dot(g, _as_bf16(w2[f * FH // 2:(f + 1) * FH // 2, :]),
                       preferred_element_type=f32)

    def attn(qkv, g, store):
        for i in range(G):
            o = _attend(qkv[:, i * E:(i + 1) * E], qkv[:, (G + i) * E:(G + i + 1) * E],
                        qkv[:, (2 * G + i) * E:(2 * G + i + 1) * E], mask, scale)
            store(g * G + i, o.astype(bf16))

    def store_a(h, o):
        o_a[:, h * E:(h + 1) * E] = o[0:SEG]
        o_b[8:16, h * E:(h + 1) * E] = o[SEG:L]

    def store_b(h, o):
        o_b[0:8, h * E:(h + 1) * E] = o[0:M]
        o_b[16:48, h * E:(h + 1) * E] = o[M:L]

    def attn_pass(proj, store, fillers, early=None):
        NG = H // G
        res = []
        cur = proj(0)
        for g in range(NG):
            if g + 1 < NG:
                nxt = proj(g + 1)
            else:
                nxt = None
                res.extend(f() for f in fillers[:1])
            if g == 1 and early is not None:
                early()
            attn(cur, g, store)
            cur = nxt
        for f in fillers[1:]:
            res.append(f())
        return res

    def dstep(j, mem, with_mlp=True):
        slot = j % 2
        xs = j % (LAG + 1)
        xq = (j + 1) % (LAG + 1)
        base = j * R if isinstance(j, int) else pl.multiple_of(j * R, R)

        if with_mlp:
            @pl.when(j >= LAG + 2)
            def _():
                out_cp(j - LAG - 2).wait()

        hb = hbuf[slot]
        st = {}

        def early():
            if with_mlp:
                xp = x1[xq].astype(f32)
                st["xp"] = xp
                st["h2"] = _layernorm_mod(xp, cb1, sb).astype(bf16)
            prep_h(jnp.minimum(j + 1, nblk - 1))

        lhs_a = jnp.concatenate([mem, hb[0:SEG - 8]], axis=0).astype(bf16)
        lhs_b_rest = hb[SEG:R - 8]
        p0 = j * 16 if isinstance(j, int) else pl.multiple_of(j * 16, 16)

        def proj(lhs, g, off):
            w = jnp.concatenate(wgroup(0, g) + wgroup(1, g) + wgroup(2, g), axis=1)
            qkv = jnp.dot(lhs, _as_bf16(w), preferred_element_type=f32).astype(bf16)
            return jnp.concatenate([qkv, pre[g, pl.ds(p0 + off, 8), :]], axis=0)

        proj_a = lambda g: proj(lhs_a, g, 0)

        fill = [lambda: mlp_up(st["h2"], 0), lambda: mlp_up(st["h2"], 1)] if with_mlp else []
        gs = attn_pass(proj_a, store_a, fill, early)
        r = jnp.dot(o_a[...], _as_bf16(wo[...]), preferred_element_type=f32)
        if with_mlp:
            y1 = mlp_down(gs[0], 0)
        mem_b = r[0:M]
        xb = xv[pl.ds(base, R), :].astype(f32)
        x1[xs, 0:SEG - 8, :] = (xb[0:SEG - 8] + ga * r[M:SEG]).astype(bf16)
        lhs_b = jnp.concatenate([mem_b, lhs_b_rest], axis=0).astype(bf16)

        proj_b = lambda g: proj(lhs_b, g, 8)
        fill = [lambda: mlp_down(gs[1], 1)] if with_mlp else []
        ys = attn_pass(proj_b, store_b, fill)
        if with_mlp:
            obuf[(j - LAG) % 2] = (st["xp"] + gb * (y1 + ys[0] + b2)).astype(bf16)
        r = jnp.dot(o_b[...], _as_bf16(wo[...]), preferred_element_type=f32)
        x1[xs, SEG - 8:R, :] = (xb[SEG - 8:R] + ga * r[M:M + SEG + 8]).astype(bf16)
        if with_mlp:
            out_cp(j - LAG).start()
        return r[0:M]

    prep_h(0)
    mem1 = lax.fori_loop(0, LAG, lambda j, m: dstep(j, m, with_mlp=False),
                         mem0_ref[...].astype(f32))
    sb = mod_vec(3)
    cb1 = 1.0 + mod_vec(4)
    gb = mod_vec(5)
    w1_cp.wait()
    w2_cp.wait()
    b2 = b2_ref[...].astype(f32)
    lax.fori_loop(LAG, nblk, dstep, mem1)

    out_cp(nblk - LAG - 2).wait()
    out_cp(nblk - LAG - 1).wait()
    tail = list(range(nblk - LAG, nblk))
    xp = jnp.concatenate([x1[i % (LAG + 1)] for i in tail], axis=0).astype(f32)
    h2 = _layernorm_mod(xp, cb1, sb).astype(bf16)
    y = mlp_down(mlp_up(h2, 0), 0) + mlp_down(mlp_up(h2, 1), 1)
    otail[...] = (xp + gb * (y + b2)).astype(bf16)
    cp = pltpu.make_async_copy(otail, out_hbm.at[pl.ds((nblk - LAG) * R, LAG * R)], osems.at[0])
    cp.start()
    cp.wait()


@functools.partial(jax.jit, static_argnames=("A_seg_len",))
def pallas_adaLN_cond__memory_aug_recurrent_mem_tr__dense_activation_gelu__prompt_kernel(
    A_x, A_mem0, A_Wq, A_Wk, A_Wv, A_Wo, A_seg_len, B_x, B_w1, B_b1, B_w2, B_b2, c, w_mod,
):
    del B_x
    B, S, D = A_x.shape
    _, H, E = A_Wq.shape
    M = A_mem0.shape[1]
    F = B_w1.shape[1]
    SEG = A_seg_len
    assert B == 1 and M == 8 and SEG == 32 and S % (2 * SEG) == 0 and H % 2 == 0
    DC, NSLOT, LAG = 256, 4, 1
    bf16, i32, f32 = jnp.bfloat16, jnp.int32, jnp.float32

    hbm = pl.BlockSpec(memory_space=pl.ANY)
    vmem = pl.BlockSpec(memory_space=pltpu.VMEM)
    kern = functools.partial(_kernel, S=S, D=D, H=H, E=E, M=M, SEG=SEG, F=F,
                             DC=DC, NSLOT=NSLOT, LAG=LAG)
    c8 = jnp.broadcast_to(c, (16, D))
    out = pl.pallas_call(
        kern,
        out_shape=jax.ShapeDtypeStruct((S, D), bf16),
        in_specs=[hbm, hbm, vmem, hbm, hbm, hbm, hbm, hbm, vmem, hbm, vmem, vmem, hbm],
        out_specs=hbm,
        scratch_shapes=[
            pltpu.VMEM((2, H // 2 * (D // 2 + 8), E), i32),
            pltpu.VMEM((2, H // 2 * (D // 2 + 8), E), i32),
            pltpu.VMEM((2, H // 2 * (D // 2 + 8), E), i32),
            pltpu.VMEM((H * E // 2, D), i32),
            pltpu.VMEM((D // 2, F), i32),
            pltpu.VMEM((F // 2, D), i32),
            pltpu.VMEM((6, D // 2, D), i32),
            pltpu.VMEM((NSLOT, DC * H // 2, E), i32),
            pltpu.VMEM((S, D), bf16),
            pltpu.VMEM((LAG + 1, 2 * SEG, D), bf16),
            pltpu.VMEM((2, 2 * SEG, D), f32),
            pltpu.VMEM((S // SEG, 8, D), bf16),
            pltpu.VMEM((S // SEG * 4, D), i32),
            pltpu.VMEM((H // 4, S // SEG * 8, 12 * E), bf16),
            pltpu.VMEM((SEG, H * E), bf16),
            pltpu.VMEM((SEG + 16, H * E), bf16),
            pltpu.VMEM((2, 2 * SEG, D), bf16),
            pltpu.VMEM((LAG * 2 * SEG, D), bf16),
            pltpu.SemaphoreType.DMA((12,)),
            pltpu.SemaphoreType.DMA((NSLOT,)),
            pltpu.SemaphoreType.DMA((2,)),
        ],
        compiler_params=pltpu.CompilerParams(vmem_limit_bytes=110 * 1024 * 1024),
    )(A_x.reshape(S, D), A_x.reshape(S // SEG, SEG, D), A_mem0.reshape(M, D),
      A_Wq.reshape(D * H, E), A_Wk.reshape(D * H, E), A_Wv.reshape(D * H, E),
      A_Wo.reshape(H * E, D), B_w1, B_b1.reshape(1, F), B_w2, B_b2.reshape(1, D),
      c8, w_mod)
    return out.reshape(B, S, D)
```

```python
import functools
import math

import jax
import jax.numpy as jnp
from jax import lax
import jax.experimental.pallas as pl
import jax.experimental.pallas.tpu as pltpu

_EPS = 1e-5
_GELU_C = math.sqrt(2.0 / math.pi)


def _as_bf16(w_i32):
    return pltpu.bitcast(w_i32, jnp.bfloat16)


def _layernorm_mod(x, scale1, shift):
    m = jnp.mean(x, axis=-1, keepdims=True)
    d = x - m
    v = jnp.mean(d * d, axis=-1, keepdims=True)
    return d * lax.rsqrt(v + _EPS) * scale1 + shift


def _gelu(a):
    return 0.5 * a * (1.0 + jnp.tanh(_GELU_C * (a + 0.044715 * (a * a * a))))


def _probs(q, k, mask, scale):
    s = lax.dot_general(q, k, (((1,), (1,)), ((), ())),
                        preferred_element_type=jnp.float32) * scale
    s = jnp.where(mask, s, -1e9)
    m = jnp.max(s, axis=-1, keepdims=True)
    e = jnp.exp(s - m)
    return (e / jnp.sum(e, axis=-1, keepdims=True)).astype(jnp.bfloat16)


def _kernel(x_hbm, x3_hbm, mem0_ref, wq_hbm, wk_hbm, wv_hbm, wo_hbm, w1_hbm, b1_ref,
            w2_hbm, b2_ref, c_ref, wmod_hbm, out_hbm,
            wq, wk, wv, wo, w1, w2, wmod, stage, xv, x1, hbuf, xpre, hpre, pre, o_a, o_b, obuf, otail,
            sems, ssems, osems, *, S, D, H, E, M, SEG, F, DC, NSLOT, LAG):
    i32, bf16, f32 = jnp.int32, jnp.bfloat16, jnp.float32
    scale = E ** -0.5
    HP = H // 2
    L = M + SEG
    G = 4

    wmod_i = wmod_hbm.bitcast(i32)
    mod_cp = [pltpu.make_async_copy(wmod_i.at[:, pl.ds(j * D, D)], wmod.at[j], sems.at[j])
              for j in range(6)]
    x_cp = pltpu.make_async_copy(x_hbm, xv, sems.at[6])
    wo_cp = pltpu.make_async_copy(wo_hbm.bitcast(i32), wo, sems.at[7])
    w1_cp = pltpu.make_async_copy(w1_hbm.bitcast(i32), w1, sems.at[8])
    w2_cp = pltpu.make_async_copy(w2_hbm.bitcast(i32), w2, sems.at[9])

    srcs = [wq_hbm.bitcast(i32), wk_hbm.bitcast(i32), wv_hbm.bitcast(i32)]
    chunks = [(t, cidx) for t in range(3) for cidx in range(D // DC)]

    def stage_cp(n):
        t, cidx = chunks[n]
        return pltpu.make_async_copy(srcs[t].at[pl.ds(cidx * DC * HP, DC * HP)],
                                     stage.at[n % NSLOT], ssems.at[n % NSLOT])

    NS = S // SEG
    PB = NS * 8
    xb_cp = pltpu.make_async_copy(x3_hbm.at[:, pl.ds(SEG - 8, 8), :], xpre, sems.at[11])
    xb_cp.start()
    mod_cp[0].start()
    mod_cp[1].start()
    for n in range(NSLOT):
        stage_cp(n).start()

    cv = c_ref[...].astype(f32)
    sc = (cv * jax.nn.sigmoid(cv)).astype(bf16)

    def mod_vec(j):
        mod_cp[j].wait()
        r = jnp.dot(sc, _as_bf16(wmod[j]), preferred_element_type=f32)
        return r[0:1, :].astype(bf16).astype(f32)

    sa = mod_vec(0)
    ca1 = 1.0 + mod_vec(1)
    xb_cp.wait()
    hpre[...] = pltpu.bitcast(
        _layernorm_mod(xpre[...].reshape(PB, D).astype(f32), ca1, sa).astype(bf16), i32)
    wts = ((wq.at[0], wq.at[1]), (wk.at[0], wk.at[1]), (wv.at[0], wv.at[1]))

    per = D // DC
    W = G * E

    PITCH = D // 2 + 8

    def repack(n):
        t, cidx = chunks[n]
        slot = n % NSLOT
        stage_cp(n).wait()
        w_even, w_odd = wts[t]

        def body(q, carry):
            for u in range(8):
                pp = q * 8 + u
                a = stage[slot, pl.ds(pl.multiple_of(pp * 2 * HP, 2 * HP), HP), :]
                b = stage[slot, pl.ds(pl.multiple_of(pp * 2 * HP + HP, HP), HP), :]
                lo = (a & 0xFFFF) | (b << 16)
                hi = lax.shift_right_logical(a, 16) | (b & jnp.int32(-65536))
                dst = pl.ds(cidx * DC // 2 + pp, HP, stride=PITCH)
                w_even[dst, :] = lo
                w_odd[dst, :] = hi
            return carry

        lax.fori_loop(0, DC // 16, body, 0)
        if n + NSLOT < len(chunks):
            stage_cp(n + NSLOT).start()

    def wgroup(t, g):
        w_even, w_odd = wts[t]
        parts = []
        for i in range(G // 2):
            hp = g * (G // 2) + i
            r0 = hp * PITCH if isinstance(hp, int) else pl.multiple_of(hp * PITCH, 8)
            parts += [w_even[pl.ds(r0, D // 2), :], w_odd[pl.ds(r0, D // 2), :]]
        return parts

    for t in range(3):
        for n in range(t * per, (t + 1) * per):
            repack(n)
        if t == 0:
            x_cp.start()
            wo_cp.start()
            mod_cp[2].start()
        if t == 1:
            w1_cp.start()
            w2_cp.start()
            for j in range(3, 6):
                mod_cp[j].start()

        def bulk(g, carry, t=t):
            w = jnp.concatenate(wgroup(t, g), axis=1)
            pre[g, :, pl.ds(t * W, W)] = jnp.dot(
                _as_bf16(hpre[...]), _as_bf16(w), preferred_element_type=f32).astype(bf16)
            return carry

        lax.fori_loop(0, H // G, bulk, 0)

    wo_cp.wait()
    x_cp.wait()
    ga = mod_vec(2)

    ri = lax.broadcasted_iota(i32, (L, L), 0)
    ci = lax.broadcasted_iota(i32, (L, L), 1)
    mask = (ri < M) | (ri >= ci)
    R = 2 * SEG
    nblk = S // R
    FH = F // 2

    def out_cp(i):
        return pltpu.make_async_copy(obuf.at[i % 2], out_hbm.at[pl.ds(i * R, R)], osems.at[i % 2])

    def prep_h(i):
        xb = xv[pl.ds(pl.multiple_of(i * R, R), R), :].astype(f32)
        hbuf[i % 2] = _layernorm_mod(xb, ca1, sa)

    def mlp_up(h2, f):
        a = jnp.dot(h2, _as_bf16(w1[:, f * FH:(f + 1) * FH]), preferred_element_type=f32)
        a = a + b1_ref[:, f * FH:(f + 1) * FH].astype(f32)
        return _gelu(a).astype(bf16)

    def mlp_down(g, f, half=None):
        r0, r1 = f * FH // 2, (f + 1) * FH // 2
        if half is not None:
            mid = (r0 + r1) // 2
            r0, r1 = ((r0, mid), (mid, r1))[half]
            g = g[:, half * (FH // 2):(half + 1) * (FH // 2)]
        return jnp.dot(g, _as_bf16(w2[r0:r1, :]), preferred_element_type=f32)

    def attn_qk(qkv):
        return [_probs(qkv[:, i * E:(i + 1) * E], qkv[:, (G + i) * E:(G + i + 1) * E], mask, scale)
                for i in range(G)]

    def attn_pv(qkv, ps, g, store):
        for i in range(G):
            o = jnp.dot(ps[i], qkv[:, (2 * G + i) * E:(2 * G + i + 1) * E],
                        preferred_element_type=f32)
            store(g * G + i, o.astype(bf16))

    def store_a(h, o):
        o_a[:, h * E:(h + 1) * E] = o[0:SEG]
        o_b[8:16, h * E:(h + 1) * E] = o[SEG:L]

    def store_b(h, o):
        o_b[0:8, h * E:(h + 1) * E] = o[0:M]
        o_b[16:48, h * E:(h + 1) * E] = o[M:L]

    def attn_pass(proj, store, fillers, early=None):
        NG = H // G
        res = []
        fillers = list(fillers)
        qkv = {0: proj(0)}
        ps = {}
        for g in range(NG + 1):
            if g + 1 < NG:
                qkv[g + 1] = proj(g + 1)
            elif fillers:
                res.append(fillers.pop(0)())
            if g == 1 and early is not None:
                early()
            if g >= 1:
                attn_pv(qkv[g - 1], ps[g - 1], g - 1, store)
            if g < NG:
                ps[g] = attn_qk(qkv[g])
        return res

    def dstep(j, mem, with_mlp=True):
        slot = j % 2
        xs = j % (LAG + 1)
        xq = (j + 1) % (LAG + 1)
        base = j * R if isinstance(j, int) else pl.multiple_of(j * R, R)

        if with_mlp:
            @pl.when(j >= LAG + 2)
            def _():
                out_cp(j - LAG - 2).wait()

        hb = hbuf[slot]
        st = {}

        def early():
            if with_mlp:
                xp = x1[xq].astype(f32)
                st["xp"] = xp
                st["h2"] = _layernorm_mod(xp, cb1, sb).astype(bf16)
            prep_h(jnp.minimum(j + 1, nblk - 1))

        lhs_a = jnp.concatenate([mem, hb[0:SEG - 8]], axis=0).astype(bf16)
        lhs_b_rest = hb[SEG:R - 8]
        p0 = j * 16 if isinstance(j, int) else pl.multiple_of(j * 16, 16)

        def proj(lhs, g, off):
            w = jnp.concatenate(wgroup(0, g) + wgroup(1, g) + wgroup(2, g), axis=1)
            qkv = jnp.dot(lhs, _as_bf16(w), preferred_element_type=f32).astype(bf16)
            return jnp.concatenate([qkv, pre[g, pl.ds(p0 + off, 8), :]], axis=0)

        proj_a = lambda g: proj(lhs_a, g, 0)

        fill = [lambda: mlp_up(st["h2"], 0), lambda: mlp_up(st["h2"], 1)] if with_mlp else []
        gs = attn_pass(proj_a, store_a, fill, early)
        r = jnp.dot(o_a[...], _as_bf16(wo[...]), preferred_element_type=f32)
        if with_mlp:
            y1 = mlp_down(gs[0], 0, 0)
        mem_b = r[0:M]
        xb = xv[pl.ds(base, R), :].astype(f32)
        x1[xs, 0:SEG - 8, :] = (xb[0:SEG - 8] + ga * r[M:SEG]).astype(bf16)
        lhs_b = jnp.concatenate([mem_b, lhs_b_rest], axis=0).astype(bf16)

        proj_b = lambda g: proj(lhs_b, g, 8)
        fill = [lambda: mlp_down(gs[0], 0, 1), lambda: mlp_down(gs[1], 1)] if with_mlp else []
        ys = attn_pass(proj_b, store_b, fill)
        if with_mlp:
            obuf[(j - LAG) % 2] = (st["xp"] + gb * (y1 + ys[0] + ys[1] + b2)).astype(bf16)
        r = jnp.dot(o_b[...], _as_bf16(wo[...]), preferred_element_type=f32)
        x1[xs, SEG - 8:R, :] = (xb[SEG - 8:R] + ga * r[M:M + SEG + 8]).astype(bf16)
        if with_mlp:
            out_cp(j - LAG).start()
        return r[0:M]

    prep_h(0)
    mem1 = lax.fori_loop(0, LAG, lambda j, m: dstep(j, m, with_mlp=False),
                         mem0_ref[...].astype(f32))
    sb = mod_vec(3)
    cb1 = 1.0 + mod_vec(4)
    gb = mod_vec(5)
    w1_cp.wait()
    w2_cp.wait()
    b2 = b2_ref[...].astype(f32)
    lax.fori_loop(LAG, nblk, dstep, mem1)

    out_cp(nblk - LAG - 2).wait()
    out_cp(nblk - LAG - 1).wait()
    tail = list(range(nblk - LAG, nblk))
    xp = jnp.concatenate([x1[i % (LAG + 1)] for i in tail], axis=0).astype(f32)
    h2 = _layernorm_mod(xp, cb1, sb).astype(bf16)
    y = mlp_down(mlp_up(h2, 0), 0) + mlp_down(mlp_up(h2, 1), 1)
    otail[...] = (xp + gb * (y + b2)).astype(bf16)
    cp = pltpu.make_async_copy(otail, out_hbm.at[pl.ds((nblk - LAG) * R, LAG * R)], osems.at[0])
    cp.start()
    cp.wait()


@functools.partial(jax.jit, static_argnames=("A_seg_len",))
def pallas_adaLN_cond__memory_aug_recurrent_mem_tr__dense_activation_gelu__prompt_kernel(
    A_x, A_mem0, A_Wq, A_Wk, A_Wv, A_Wo, A_seg_len, B_x, B_w1, B_b1, B_w2, B_b2, c, w_mod,
):
    del B_x
    B, S, D = A_x.shape
    _, H, E = A_Wq.shape
    M = A_mem0.shape[1]
    F = B_w1.shape[1]
    SEG = A_seg_len
    assert B == 1 and M == 8 and SEG == 32 and S % (2 * SEG) == 0 and H % 2 == 0
    DC, NSLOT, LAG = 256, 4, 1
    bf16, i32, f32 = jnp.bfloat16, jnp.int32, jnp.float32

    hbm = pl.BlockSpec(memory_space=pl.ANY)
    vmem = pl.BlockSpec(memory_space=pltpu.VMEM)
    kern = functools.partial(_kernel, S=S, D=D, H=H, E=E, M=M, SEG=SEG, F=F,
                             DC=DC, NSLOT=NSLOT, LAG=LAG)
    c8 = jnp.broadcast_to(c, (16, D))
    out = pl.pallas_call(
        kern,
        out_shape=jax.ShapeDtypeStruct((S, D), bf16),
        in_specs=[hbm, hbm, vmem, hbm, hbm, hbm, hbm, hbm, vmem, hbm, vmem, vmem, hbm],
        out_specs=hbm,
        scratch_shapes=[
            pltpu.VMEM((2, H // 2 * (D // 2 + 8), E), i32),
            pltpu.VMEM((2, H // 2 * (D // 2 + 8), E), i32),
            pltpu.VMEM((2, H // 2 * (D // 2 + 8), E), i32),
            pltpu.VMEM((H * E // 2, D), i32),
            pltpu.VMEM((D // 2, F), i32),
            pltpu.VMEM((F // 2, D), i32),
            pltpu.VMEM((6, D // 2, D), i32),
            pltpu.VMEM((NSLOT, DC * H // 2, E), i32),
            pltpu.VMEM((S, D), bf16),
            pltpu.VMEM((LAG + 1, 2 * SEG, D), bf16),
            pltpu.VMEM((2, 2 * SEG, D), f32),
            pltpu.VMEM((S // SEG, 8, D), bf16),
            pltpu.VMEM((S // SEG * 4, D), i32),
            pltpu.VMEM((H // 4, S // SEG * 8, 12 * E), bf16),
            pltpu.VMEM((SEG, H * E), bf16),
            pltpu.VMEM((SEG + 16, H * E), bf16),
            pltpu.VMEM((2, 2 * SEG, D), bf16),
            pltpu.VMEM((LAG * 2 * SEG, D), bf16),
            pltpu.SemaphoreType.DMA((12,)),
            pltpu.SemaphoreType.DMA((NSLOT,)),
            pltpu.SemaphoreType.DMA((2,)),
        ],
        compiler_params=pltpu.CompilerParams(vmem_limit_bytes=110 * 1024 * 1024),
    )(A_x.reshape(S, D), A_x.reshape(S // SEG, SEG, D), A_mem0.reshape(M, D),
      A_Wq.reshape(D * H, E), A_Wk.reshape(D * H, E), A_Wv.reshape(D * H, E),
      A_Wo.reshape(H * E, D), B_w1, B_b1.reshape(1, F), B_w2, B_b2.reshape(1, D),
      c8, w_mod)
    return out.reshape(B, S, D)
```

```python
import functools
import math

import jax
import jax.numpy as jnp
from jax import lax
import jax.experimental.pallas as pl
import jax.experimental.pallas.tpu as pltpu

_EPS = 1e-5
_GELU_C = math.sqrt(2.0 / math.pi)


def _as_bf16(w_i32):
    return pltpu.bitcast(w_i32, jnp.bfloat16)


def _layernorm_mod(x, scale1, shift):
    m = jnp.mean(x, axis=-1, keepdims=True)
    d = x - m
    v = jnp.mean(d * d, axis=-1, keepdims=True)
    return d * lax.rsqrt(v + _EPS) * scale1 + shift


def _gelu(a):
    return 0.5 * a * (1.0 + jnp.tanh(_GELU_C * (a + 0.044715 * (a * a * a))))


def _probs(q, k, mask, scale):
    s = lax.dot_general(q, k, (((1,), (1,)), ((), ())),
                        preferred_element_type=jnp.float32) * scale
    s = jnp.where(mask, s, -1e9)
    m = jnp.max(s, axis=-1, keepdims=True)
    e = jnp.exp(s - m)
    return (e / jnp.sum(e, axis=-1, keepdims=True)).astype(jnp.bfloat16)


def _kernel(x_hbm, x3_hbm, mem0_ref, wq_hbm, wk_hbm, wv_hbm, wo_hbm, w1_hbm, b1_ref,
            w2_hbm, b2_ref, c_ref, wmod_hbm, out_hbm,
            wq, wk, wv, wo, w1, w2, wmod, stage, xv, x1, hbuf, xpre, hpre, pre, o_a, o_b, obuf, otail,
            sems, ssems, osems, *, S, D, H, E, M, SEG, F, DC, NSLOT, LAG):
    i32, bf16, f32 = jnp.int32, jnp.bfloat16, jnp.float32
    scale = E ** -0.5
    HP = H // 2
    L = M + SEG
    G = 4

    wmod_i = wmod_hbm.bitcast(i32)
    mod_cp = [pltpu.make_async_copy(wmod_i.at[:, pl.ds(j * D, D)], wmod.at[j], sems.at[j])
              for j in range(6)]
    x_cp = pltpu.make_async_copy(x_hbm, xv, sems.at[6])
    wo_cp = pltpu.make_async_copy(wo_hbm.bitcast(i32), wo, sems.at[7])
    w1_cp = pltpu.make_async_copy(w1_hbm.bitcast(i32), w1, sems.at[8])
    w2_cp = pltpu.make_async_copy(w2_hbm.bitcast(i32), w2, sems.at[9])

    srcs = [wq_hbm.bitcast(i32), wk_hbm.bitcast(i32), wv_hbm.bitcast(i32)]
    chunks = [(t, cidx) for t in range(3) for cidx in range(D // DC)]

    def stage_cp(n):
        t, cidx = chunks[n]
        return pltpu.make_async_copy(srcs[t].at[pl.ds(cidx * DC * HP, DC * HP)],
                                     stage.at[n % NSLOT], ssems.at[n % NSLOT])

    NS = S // SEG
    PB = NS * 8
    xb_cp = pltpu.make_async_copy(x3_hbm.at[:, pl.ds(SEG - 8, 8), :], xpre, sems.at[11])
    xb_cp.start()
    mod_cp[0].start()
    mod_cp[1].start()
    for n in range(NSLOT):
        stage_cp(n).start()

    cv = jnp.broadcast_to(c_ref[...].astype(f32), (16, D))
    sc = (cv * jax.nn.sigmoid(cv)).astype(bf16)

    def mod_vec(j):
        mod_cp[j].wait()
        r = jnp.dot(sc, _as_bf16(wmod[j]), preferred_element_type=f32)
        return r[0:1, :].astype(bf16).astype(f32)

    sa = mod_vec(0)
    ca1 = 1.0 + mod_vec(1)
    xb_cp.wait()
    hpre[...] = pltpu.bitcast(
        _layernorm_mod(xpre[...].reshape(PB, D).astype(f32), ca1, sa).astype(bf16), i32)
    wts = ((wq.at[0], wq.at[1]), (wk.at[0], wk.at[1]), (wv.at[0], wv.at[1]))

    per = D // DC
    W = G * E

    PITCH = D // 2 + 8

    def repack_rows(t, slot, cidx, pp):
        w_even, w_odd = wts[t]
        a = stage[slot, pl.ds(pl.multiple_of(pp * 2 * HP, 2 * HP), HP), :]
        b = stage[slot, pl.ds(pl.multiple_of(pp * 2 * HP + HP, HP), HP), :]
        lo = (a & 0xFFFF) | (b << 16)
        hi = lax.shift_right_logical(a, 16) | (b & jnp.int32(-65536))
        dst = pl.ds(cidx * (DC // 2) + pp, HP, stride=PITCH)
        w_even[dst, :] = lo
        w_odd[dst, :] = hi

    def repack(n):
        t, cidx = chunks[n]
        stage_cp(n).wait()

        def body(q, carry):
            for u in range(8):
                repack_rows(t, n % NSLOT, cidx, q * 8 + u)
            return carry

        lax.fori_loop(0, DC // 16, body, 0)
        stage_cp(n + NSLOT).start()

    def wgroup(t, g):
        w_even, w_odd = wts[t]
        parts = []
        for i in range(G // 2):
            hp = g * (G // 2) + i
            r0 = hp * PITCH if isinstance(hp, int) else pl.multiple_of(hp * PITCH, 8)
            parts += [w_even[pl.ds(r0, D // 2), :], w_odd[pl.ds(r0, D // 2), :]]
        return parts

    assert NSLOT == per
    for n in range(per):
        repack(n)
    GPI = (H // G) // per
    for t in range(3):
        if t == 1:
            x_cp.start()
            wo_cp.start()
            mod_cp[2].start()
            w1_cp.start()
            w2_cp.start()
            for j in range(3, 6):
                mod_cp[j].start()

        def bulk(c, carry, t=t):
            if t < 2:
                src = srcs[t + 1].at[pl.ds(pl.multiple_of(c * DC * HP, DC * HP), DC * HP)]
                pltpu.make_async_copy(src, stage.at[c], ssems.at[c]).wait()
            for u in range(GPI):
                g = c * GPI + u
                if t < 2 and u == 0:
                    for pp in range(DC // 2):
                        repack_rows(t + 1, c, c, pp)
                w = jnp.concatenate(wgroup(t, g), axis=1)
                pre[g, :, pl.ds(t * W, W)] = jnp.dot(
                    _as_bf16(hpre[...]), _as_bf16(w), preferred_element_type=f32).astype(bf16)
            if t < 1:
                src = srcs[2].at[pl.ds(pl.multiple_of(c * DC * HP, DC * HP), DC * HP)]
                pltpu.make_async_copy(src, stage.at[c], ssems.at[c]).start()
            return carry

        lax.fori_loop(0, per, bulk, 0)

    wo_cp.wait()
    x_cp.wait()
    ga = mod_vec(2)

    ri = lax.broadcasted_iota(i32, (L, L), 0)
    ci = lax.broadcasted_iota(i32, (L, L), 1)
    mask = (ri < M) | (ri >= ci)
    R = 2 * SEG
    nblk = S // R
    FH = F // 2

    def out_cp(i):
        return pltpu.make_async_copy(obuf.at[i % 2], out_hbm.at[pl.ds(i * R, R)], osems.at[i % 2])

    def prep_h(i):
        xb = xv[pl.ds(pl.multiple_of(i * R, R), R), :].astype(f32)
        hbuf[i % 2] = _layernorm_mod(xb, ca1, sa)

    def mlp_up(h2, f):
        a = jnp.dot(h2, _as_bf16(w1[:, f * FH:(f + 1) * FH]), preferred_element_type=f32)
        a = a + b1v[:, f * FH:(f + 1) * FH]
        return _gelu(a).astype(bf16)

    def mlp_down(g, f, half=None):
        r0, r1 = f * FH // 2, (f + 1) * FH // 2
        if half is not None:
            mid = (r0 + r1) // 2
            r0, r1 = ((r0, mid), (mid, r1))[half]
            g = g[:, half * (FH // 2):(half + 1) * (FH // 2)]
        return jnp.dot(g, _as_bf16(w2[r0:r1, :]), preferred_element_type=f32)

    def attn_qk(qkv):
        return [_probs(qkv[:, i * E:(i + 1) * E], qkv[:, (G + i) * E:(G + i + 1) * E], mask, scale)
                for i in range(G)]

    def attn_pv(qkv, ps, g, store):
        for i in range(G):
            o = jnp.dot(ps[i], qkv[:, (2 * G + i) * E:(2 * G + i + 1) * E],
                        preferred_element_type=f32)
            store(g * G + i, o.astype(bf16))

    def store_a(h, o):
        o_a[:, h * E:(h + 1) * E] = o[0:SEG]
        o_b[8:16, h * E:(h + 1) * E] = o[SEG:L]

    def store_b(h, o):
        o_b[0:8, h * E:(h + 1) * E] = o[0:M]
        o_b[16:48, h * E:(h + 1) * E] = o[M:L]

    def attn_pass(proj, store, fillers, early=None):
        NG = H // G
        res = []
        fillers = list(fillers)
        qkv = {0: proj(0)}
        ps = {}
        for g in range(NG + 1):
            if g + 1 < NG:
                qkv[g + 1] = proj(g + 1)
            elif fillers:
                res.append(fillers.pop(0)())
            if g == 1 and early is not None:
                early()
            if g >= 1:
                attn_pv(qkv[g - 1], ps[g - 1], g - 1, store)
            if g < NG:
                ps[g] = attn_qk(qkv[g])
        return res

    def dstep(j, mem, with_mlp=True):
        slot = j % 2
        xs = j % (LAG + 1)
        xq = (j + 1) % (LAG + 1)
        base = j * R if isinstance(j, int) else pl.multiple_of(j * R, R)

        if with_mlp:
            @pl.when(j >= LAG + 2)
            def _():
                out_cp(j - LAG - 2).wait()

        hb = hbuf[slot]
        st = {}

        def early():
            if with_mlp:
                xp = x1[xq].astype(f32)
                st["xp"] = xp
                st["h2"] = _layernorm_mod(xp, cb1, sb).astype(bf16)
            prep_h(jnp.minimum(j + 1, nblk - 1))

        lhs_a = jnp.concatenate([mem, hb[0:SEG - 8]], axis=0).astype(bf16)
        lhs_b_rest = hb[SEG:R - 8]
        p0 = j * 16 if isinstance(j, int) else pl.multiple_of(j * 16, 16)

        def proj(lhs, g, off):
            w = jnp.concatenate(wgroup(0, g) + wgroup(1, g) + wgroup(2, g), axis=1)
            qkv = jnp.dot(lhs, _as_bf16(w), preferred_element_type=f32).astype(bf16)
            return jnp.concatenate([qkv, pre[g, pl.ds(p0 + off, 8), :]], axis=0)

        proj_a = lambda g: proj(lhs_a, g, 0)

        fill = [lambda: mlp_up(st["h2"], 0), lambda: mlp_up(st["h2"], 1)] if with_mlp else []
        gs = attn_pass(proj_a, store_a, fill, early)
        r = jnp.dot(o_a[...], _as_bf16(wo[...]), preferred_element_type=f32)
        if with_mlp:
            y1 = mlp_down(gs[0], 0, 0)
        mem_b = r[0:M]
        xb = xv[pl.ds(base, R), :].astype(f32)
        x1[xs, 0:SEG - 8, :] = (xb[0:SEG - 8] + ga * r[M:SEG]).astype(bf16)
        lhs_b = jnp.concatenate([mem_b, lhs_b_rest], axis=0).astype(bf16)

        proj_b = lambda g: proj(lhs_b, g, 8)
        fill = [lambda: mlp_down(gs[0], 0, 1), lambda: mlp_down(gs[1], 1)] if with_mlp else []
        ys = attn_pass(proj_b, store_b, fill)
        if with_mlp:
            obuf[(j - LAG) % 2] = (st["xp"] + gb * (y1 + ys[0] + ys[1] + b2)).astype(bf16)
        r = jnp.dot(o_b[...], _as_bf16(wo[...]), preferred_element_type=f32)
        x1[xs, SEG - 8:R, :] = (xb[SEG - 8:R] + ga * r[M:M + SEG + 8]).astype(bf16)
        if with_mlp:
            out_cp(j - LAG).start()
        return r[0:M]

    prep_h(0)
    mem1 = lax.fori_loop(0, LAG, lambda j, m: dstep(j, m, with_mlp=False),
                         mem0_ref[...].astype(f32))
    sb = mod_vec(3)
    cb1 = 1.0 + mod_vec(4)
    gb = mod_vec(5)
    w1_cp.wait()
    w2_cp.wait()
    b2 = b2_ref[...].reshape(1, D).astype(f32)
    b1v = b1_ref[...].reshape(1, F).astype(f32)
    lax.fori_loop(LAG, nblk, dstep, mem1)

    out_cp(nblk - LAG - 2).wait()
    out_cp(nblk - LAG - 1).wait()
    tail = list(range(nblk - LAG, nblk))
    xp = jnp.concatenate([x1[i % (LAG + 1)] for i in tail], axis=0).astype(f32)
    h2 = _layernorm_mod(xp, cb1, sb).astype(bf16)
    y = mlp_down(mlp_up(h2, 0), 0) + mlp_down(mlp_up(h2, 1), 1)
    otail[...] = (xp + gb * (y + b2)).astype(bf16)
    cp = pltpu.make_async_copy(otail, out_hbm.at[pl.ds((nblk - LAG) * R, LAG * R)], osems.at[0])
    cp.start()
    cp.wait()


@functools.partial(jax.jit, static_argnames=("A_seg_len",))
def pallas_adaLN_cond__memory_aug_recurrent_mem_tr__dense_activation_gelu__prompt_kernel(
    A_x, A_mem0, A_Wq, A_Wk, A_Wv, A_Wo, A_seg_len, B_x, B_w1, B_b1, B_w2, B_b2, c, w_mod,
):
    del B_x
    B, S, D = A_x.shape
    _, H, E = A_Wq.shape
    M = A_mem0.shape[1]
    F = B_w1.shape[1]
    SEG = A_seg_len
    assert B == 1 and M == 8 and SEG == 32 and S % (2 * SEG) == 0 and H % 2 == 0
    DC, NSLOT, LAG = 256, 4, 1
    bf16, i32, f32 = jnp.bfloat16, jnp.int32, jnp.float32

    hbm = pl.BlockSpec(memory_space=pl.ANY)
    vmem = pl.BlockSpec(memory_space=pltpu.VMEM)
    kern = functools.partial(_kernel, S=S, D=D, H=H, E=E, M=M, SEG=SEG, F=F,
                             DC=DC, NSLOT=NSLOT, LAG=LAG)
    out = pl.pallas_call(
        kern,
        out_shape=jax.ShapeDtypeStruct((S, D), bf16),
        in_specs=[hbm, hbm, vmem, hbm, hbm, hbm, hbm, hbm, vmem, hbm, vmem, vmem, hbm],
        out_specs=hbm,
        scratch_shapes=[
            pltpu.VMEM((2, H // 2 * (D // 2 + 8), E), i32),
            pltpu.VMEM((2, H // 2 * (D // 2 + 8), E), i32),
            pltpu.VMEM((2, H // 2 * (D // 2 + 8), E), i32),
            pltpu.VMEM((H * E // 2, D), i32),
            pltpu.VMEM((D // 2, F), i32),
            pltpu.VMEM((F // 2, D), i32),
            pltpu.VMEM((6, D // 2, D), i32),
            pltpu.VMEM((NSLOT, DC * H // 2, E), i32),
            pltpu.VMEM((S, D), bf16),
            pltpu.VMEM((LAG + 1, 2 * SEG, D), bf16),
            pltpu.VMEM((2, 2 * SEG, D), f32),
            pltpu.VMEM((S // SEG, 8, D), bf16),
            pltpu.VMEM((S // SEG * 4, D), i32),
            pltpu.VMEM((H // 4, S // SEG * 8, 12 * E), bf16),
            pltpu.VMEM((SEG, H * E), bf16),
            pltpu.VMEM((SEG + 16, H * E), bf16),
            pltpu.VMEM((2, 2 * SEG, D), bf16),
            pltpu.VMEM((LAG * 2 * SEG, D), bf16),
            pltpu.SemaphoreType.DMA((12,)),
            pltpu.SemaphoreType.DMA((NSLOT,)),
            pltpu.SemaphoreType.DMA((2,)),
        ],
        compiler_params=pltpu.CompilerParams(vmem_limit_bytes=110 * 1024 * 1024),
    )(A_x.reshape(S, D), A_x.reshape(S // SEG, SEG, D), A_mem0.reshape(M, D),
      A_Wq.reshape(D * H, E), A_Wk.reshape(D * H, E), A_Wv.reshape(D * H, E),
      A_Wo.reshape(H * E, D), B_w1, B_b1, B_w2, B_b2,
      c, w_mod)
    return out.reshape(B, S, D)
```
